```python
import os as _os
_os.environ.setdefault('JAX_PLATFORMS', 'cpu')
import jax
import jax.numpy as jnp

def _softmax(x, axis=-1):
    return jax.nn.softmax(x, axis=axis)

def _gelu(x):
    return jax.nn.gelu(x, approximate=True)

def _silu(x):
    return jax.nn.silu(x)

def _sigmoid(x):
    return jax.nn.sigmoid(x)

def _layernorm(x, axis=-1, eps=1e-05):
    m = jnp.mean(x, axis=axis, keepdims=True)
    v = jnp.var(x, axis=axis, keepdims=True)
    return (x - m) / jnp.sqrt(v + eps)

def _scatter_add(tgt, idx, src, axis=0):
    return tgt.at[idx].add(src)

def _segment_sum(src, seg, n):
    return jax.ops.segment_sum(src, seg, n)

class _Rng:

    def __init__(self, key):
        self._k = key

    def _next(self):
        self._k, sub = jax.random.split(self._k)
        return sub

    def normal(self, shape):
        return jax.random.normal(self._next(), shape, dtype=jnp.bfloat16)

    def randint(self, lo, hi, shape):
        return jax.random.randint(self._next(), shape, lo, hi, dtype=jnp.int32)

    def uniform(self, shape, lo=0.0, hi=1.0):
        return jax.random.uniform(self._next(), shape, jnp.bfloat16, lo, hi)

    def permutation(self, n):
        return jax.random.permutation(self._next(), n)
kernel_name = 'adaLN_cond__grouped_kv_mqa__mixer_gmlp__prompt'

def setup_inputs():
    _rng = _Rng(jax.random.key(int.from_bytes(__import__("os").urandom(4), "little")))
    _w = lambda a: (lambda t: t.astype(jnp.bfloat16) if jnp.issubdtype(t.dtype, jnp.floating) else t)(jnp.asarray(a))

    def _A_setup():
        B, S, D, H = (1, 2048, 512, 32)
        Dh = D // H
        return {'x': _w((lambda *s: _rng.normal(s) * 0.05)(B, S, D)), 'wq': _w((lambda *s: _rng.normal(s) * 0.05)(D, H * Dh)), 'wk': _w((lambda *s: _rng.normal(s) * 0.05)(D, Dh)), 'wv': _w((lambda *s: _rng.normal(s) * 0.05)(D, Dh)), 'wo': _w((lambda *s: _rng.normal(s) * 0.05)(H * Dh, D))}
    _A_in = _A_setup()

    def _B_setup():
        B, S, D, F = (1, 2048, 512, 1792)
        Fh = F // 2
        return {'x': _w((lambda *s: _rng.normal(s) * 0.05)(B, S, D)), 'w_in': _w((lambda *s: _rng.normal(s) * 0.4)(D, 2 * Fh)), 'w_sp': _w(0.01 * (lambda *s: _rng.normal(s) * 0.4)(S, S)), 'b_sp': _w(1.0 + 0.01 * (lambda *s: _rng.normal(s) * 0.05)(S)), 'w_out': _w((lambda *s: _rng.normal(s) * 0.05)(Fh, D))}
    _B_in = _B_setup()
    return {'A_x': _A_in['x'], 'A_wq': _A_in['wq'], 'A_wk': _A_in['wk'], 'A_wv': _A_in['wv'], 'A_wo': _A_in['wo'], 'B_x': _B_in['x'], 'B_w_in': _B_in['w_in'], 'B_w_sp': _B_in['w_sp'], 'B_b_sp': _B_in['b_sp'], 'B_w_out': _B_in['w_out'], 'c': _w((lambda *s: _rng.normal(s) * 0.05)(1, 512) * 8.0), 'w_mod': _w((lambda *s: _rng.normal(s) * 0.05)(512, 6 * 512) * 512 ** (-0.5) * 8.0)}

def reference(A_x, A_wq, A_wk, A_wv, A_wo, B_x, B_w_in, B_w_sp, B_b_sp, B_w_out, c, w_mod):

    def _A_ref(x, wq, wk, wv, wo):
        B, S, D = x.shape
        H = 32
        Dh = D // H
        q = (lambda x, *d: x.transpose(*d))((x @ wq).reshape(B, S, H, Dh), 0, 2, 1, 3)
        k = x @ wk
        v = x @ wv
        scores = jnp.einsum('bhqd,bkd->bhqk', q, k) * Dh ** (-0.5)
        p = _softmax(scores, axis=-1)
        o = jnp.einsum('bhqk,bkd->bhqd', p, v)
        return (lambda x, *d: x.transpose(*d))(o, 0, 2, 1, 3).reshape(B, S, H * Dh) @ wo

    def _B_ref(x, w_in, w_sp, b_sp, w_out):
        B, S, D = x.shape
        F = w_in.shape[-1]
        Fh = F // 2
        z = _gelu(jnp.einsum('bsd,df->bsf', x, w_in))
        z1 = z[..., :Fh].copy()
        z2 = _layernorm(z[..., Fh:], axis=-1)
        g = jnp.einsum('ts,bsf->btf', w_sp, z2) + b_sp[None, :, None]
        return jnp.einsum('bsf,fd->bsd', z1 * g, w_out)
    x = A_x
    mod = (_silu(c) @ w_mod).reshape(c.shape[0], 6, 1, -1)
    sa, ca, ga, sb, cb, gb = (mod[:, 0].copy(), mod[:, 1].copy(), mod[:, 2].copy(), mod[:, 3].copy(), mod[:, 4].copy(), mod[:, 5].copy())
    h = _layernorm(x, axis=-1) * (1 + ca) + sa
    x = x + ga * _A_ref(h, A_wq, A_wk, A_wv, A_wo)
    h = _layernorm(x, axis=-1) * (1 + cb) + sb
    x = x + gb * _B_ref(h, B_w_in, B_w_sp, B_b_sp, B_w_out)
    return x
```

```python
import functools
import math

import jax
import jax.numpy as jnp
from jax import lax
import jax.experimental.pallas as pl
import jax.experimental.pallas.tpu as pltpu

f32, bf16 = jnp.float32, jnp.bfloat16
EPS = 1e-5
NT = (((1,), (1,)), ((), ()))
TN = (((0,), (0,)), ((), ()))


def _ln(x):
    m = jnp.mean(x, axis=-1, keepdims=True)
    d = x - m
    v = jnp.mean(d * d, axis=-1, keepdims=True)
    return d * lax.rsqrt(v + EPS)


def _gelu(x):
    c0 = math.sqrt(2.0 / math.pi)
    u = x * (c0 + (c0 * 0.044715) * (x * x))
    hx = 0.5 * x
    return hx + hx * jnp.tanh(u)


def _kernel(x_hbm, wq_hbm, wkt_hbm, wvt_hbm, wo_hbm, win_hbm, wsp_hbm, bsp_hbm, wout_hbm, c_hbm, wmod_hbm,
            out_hbm,
            x_v, wq_v, wkv_v, wo_v, win_v, wsp_v, bsp_v, wout_v, c_v, wmod_v,
            wqkv_s, qt_s, k_s, vt_s, s_buf, ot_s, x1_s, z1_s, z2_s, out_v, sems, osems,
            *, S, D, H, FH, QB, KC, TB, MB):
    DH = D // H
    NQ = S // QB
    NB = H * NQ
    NC = S // KC
    NT1 = S // TB

    def cp(src, dst, i):
        return pltpu.make_async_copy(src, dst, sems.at[i])

    c_cp = cp(c_hbm, c_v, 0)
    wmod_a = cp(wmod_hbm.at[:, pl.ds(0, 2 * D)], wmod_v.at[:, pl.ds(0, 2 * D)], 1)
    wq_cp = cp(wq_hbm, wq_v, 2)
    wk_cp = cp(wkt_hbm, wkv_v.at[pl.ds(0, DH), :], 3)
    wv_cp = cp(wvt_hbm, wkv_v.at[pl.ds(DH, DH), :], 4)
    wmod_b = cp(wmod_hbm.at[:, pl.ds(2 * D, 4 * D)], wmod_v.at[:, pl.ds(2 * D, 4 * D)], 5)
    wo_cp = cp(wo_hbm, wo_v, 6)
    win_cp = cp(win_hbm, win_v, 7)
    wsp_cp = cp(wsp_hbm, wsp_v, 8)
    bsp_cp = cp(bsp_hbm, bsp_v, 9)
    wout_cp = cp(wout_hbm, wout_v, 10)
    x_cps = [cp(x_hbm.at[pl.ds(t * TB, TB), :], x_v.at[pl.ds(t * TB, TB), :], 11 + t) for t in range(NT1)]

    c_cp.start(); wmod_a.start(); wq_cp.start(); wk_cp.start(); wv_cp.start()
    for d in x_cps:
        d.start()

    c_cp.wait()
    cf = c_v[...].astype(f32)
    sc = jnp.broadcast_to(cf * jax.nn.sigmoid(cf), (16, D)).astype(bf16)
    wmod_a.wait()
    mod_a = jnp.dot(sc, wmod_v[:, 0:2 * D], preferred_element_type=f32)[0:1]
    sa = mod_a[:, 0:D]
    ca1 = 1.0 + mod_a[:, D:2 * D]

    wq_cp.wait(); wk_cp.wait(); wv_cp.wait()
    wqkv_s[0:D, :] = wq_v[...].T
    wqkv_s[D:D + 2 * DH, :] = wkv_v[...]
    qscale = (DH ** -0.5) * math.log2(math.e)
    for t in range(NT1):
        x_cps[t].wait()
        if t == NT1 - 1:
            for d in (wmod_b, wo_cp, win_cp, wsp_cp, bsp_cp, wout_cp):
                d.start()
        rows = slice(t * TB, (t + 1) * TB)
        h = (_ln(x_v[rows, :].astype(f32)) * ca1 + sa).astype(bf16)
        r = lax.dot_general(wqkv_s[...], h, NT, preferred_element_type=f32)
        qt_s[:, rows] = (r[0:D] * qscale).astype(bf16)
        k_s[rows, :] = r[D:D + DH].T.astype(bf16)
        vt_s[:, rows] = r[D + DH:D + 2 * DH].astype(bf16)

    def blk(b):
        j = b // H
        h = b % H
        return pl.ds(pl.multiple_of(h * DH, DH), DH), pl.ds(pl.multiple_of(j * QB, QB), QB)

    def step(b, m_prev, do1, do2):
        if do1:
            q = qt_s[blk(b)]
            m8 = None
        if do2:
            acc = None
            l8 = None
            mb = jnp.broadcast_to(m_prev, (8, QB))
        for c in range(NC):
            rows = slice(c * KC, (c + 1) * KC)
            if do2:
                s_old = s_buf[rows, :]
            if do1:
                s = jnp.dot(k_s[rows, :], q, preferred_element_type=f32)
                mc = jnp.max(s.reshape(KC // 8, 8, QB), axis=0)
                m8 = mc if m8 is None else jnp.maximum(m8, mc)
                s_buf[rows, :] = s
            if do2:
                p = jnp.exp2(s_old.reshape(KC // 8, 8, QB) - mb[None])
                lc = jnp.sum(p, axis=0)
                l8 = lc if l8 is None else l8 + lc
                pv = jnp.dot(vt_s[:, rows], p.reshape(KC, QB).astype(bf16), preferred_element_type=f32)
                acc = pv if acc is None else acc + pv
        if do2:
            l = jnp.sum(l8, axis=0, keepdims=True)
            ot_s[blk(b - 1)] = (acc / l).astype(bf16)
        if do1:
            return jnp.max(m8, axis=0, keepdims=True)
        return m_prev

    m = step(0, None, True, False)
    m = lax.fori_loop(1, NB, lambda b, m: step(b, m, True, True), m)
    step(NB, m, False, True)

    wmod_b.wait()
    mod_b = jnp.dot(sc, wmod_v[:, 2 * D:6 * D], preferred_element_type=f32)[0:1]
    ga = mod_b[:, 0:D]
    sb = mod_b[:, D:2 * D]
    cb1 = 1.0 + mod_b[:, 2 * D:3 * D]
    gb = mod_b[:, 3 * D:4 * D]
    wo_cp.wait(); win_cp.wait()

    def phase3(i, carry):
        rows = pl.ds(pl.multiple_of(i * MB, MB), MB)
        a = lax.dot_general(ot_s[:, rows], wo_v[...], TN, preferred_element_type=f32)
        x1 = x_v[rows, :].astype(f32) + ga * a
        x1_s[rows, :] = x1
        h2 = (_ln(x1) * cb1 + sb).astype(bf16)
        z2 = _gelu(jnp.dot(h2, win_v[:, FH:2 * FH], preferred_element_type=f32))
        z2_s[rows, :] = _ln(z2).astype(bf16)
        z1 = _gelu(jnp.dot(h2, win_v[:, 0:FH], preferred_element_type=f32))
        z1_s[rows, :] = z1
        return carry
    lax.fori_loop(0, S // MB, phase3, 0)

    wsp_cp.wait(); bsp_cp.wait(); wout_cp.wait()
    bt = bsp_v[...].astype(f32).T
    o_cps = []
    for i in range(S // MB):
        rows = slice(i * MB, (i + 1) * MB)
        bcol = jnp.concatenate([bt[:, j:j + 1] for j in range(i * MB // 128, (i + 1) * MB // 128)], axis=0)
        g = jnp.dot(wsp_v[rows, :], z2_s[...], preferred_element_type=f32) + bcol
        y = jnp.dot((z1_s[rows, :] * g).astype(bf16), wout_v[...], preferred_element_type=f32)
        out_v[rows, :] = (x1_s[rows, :] + gb * y).astype(bf16)
        d = pltpu.make_async_copy(out_v.at[pl.ds(i * MB, MB), :], out_hbm.at[pl.ds(i * MB, MB), :], osems.at[i])
        d.start()
        o_cps.append(d)
    for d in o_cps:
        d.wait()


def make(QB=512, KC=128, TB=512, MB=512, flags=None):
    def fn(A_x, A_wq, A_wk, A_wv, A_wo, B_x, B_w_in, B_w_sp, B_b_sp, B_w_out, c, w_mod):
        B, S, D = A_x.shape
        H = 32
        DH = D // H
        FH = B_w_out.shape[0]
        V = pltpu.VMEM
        scratch = [
            V((S, D), bf16), V((D, D), bf16), V((2 * DH, D), bf16), V((D, D), bf16), V((D, 2 * FH), bf16),
            V((S, S), bf16), V((S // 128, 128), bf16), V((FH, D), bf16), V((1, D), bf16), V((D, 6 * D), bf16),
            V((D + 2 * DH, D), bf16), V((D, S), bf16), V((S, DH), bf16), V((DH, S), bf16), V((S, QB), f32),
            V((D, S), bf16), V((S, D), f32), V((S, FH), f32), V((S, FH), bf16), V((S, D), bf16),
            pltpu.SemaphoreType.DMA((11 + S // TB,)), pltpu.SemaphoreType.DMA((S // MB,)),
        ]
        out = pl.pallas_call(
            functools.partial(_kernel, S=S, D=D, H=H, FH=FH, QB=QB, KC=KC, TB=TB, MB=MB),
            out_shape=jax.ShapeDtypeStruct((S, D), A_x.dtype),
            in_specs=[pl.BlockSpec(memory_space=pl.ANY)] * 11,
            out_specs=pl.BlockSpec(memory_space=pl.ANY),
            scratch_shapes=scratch,
            compiler_params=pltpu.CompilerParams(vmem_limit_bytes=100 * 2**20, flags=flags),
            name='fused',
        )(A_x.reshape(S, D), A_wq, A_wk.T, A_wv.T, A_wo, B_w_in, B_w_sp, B_b_sp.reshape(S // 128, 128), B_w_out, c, w_mod)
        return out.reshape(B, S, D)
    return fn


@jax.jit
def pallas_adaLN_cond__grouped_kv_mqa__mixer_gmlp__prompt_kernel(
    A_x: jax.Array,
    A_wq: jax.Array,
    A_wk: jax.Array,
    A_wv: jax.Array,
    A_wo: jax.Array,
    B_x: jax.Array,
    B_w_in: jax.Array,
    B_w_sp: jax.Array,
    B_b_sp: jax.Array,
    B_w_out: jax.Array,
    c: jax.Array,
    w_mod: jax.Array,
):
    return make()(A_x, A_wq, A_wk, A_wv, A_wo, B_x, B_w_in, B_w_sp, B_b_sp, B_w_out, c, w_mod)
```

```python
import functools
import math

import jax
import jax.numpy as jnp
from jax import lax
import jax.experimental.pallas as pl
import jax.experimental.pallas.tpu as pltpu

f32, bf16, u32 = jnp.float32, jnp.bfloat16, jnp.uint32
EPS = 1e-5
NT = (((1,), (1,)), ((), ()))
T = 128
NL = 4
HS = T // 8
W_SLOTS = T // 16
L_MIN, L_MAX = 2.0 ** -40, 2.0 ** 80


def _ln(x):
    m = jnp.mean(x, axis=-1, keepdims=True)
    d = x - m
    v = jnp.mean(d * d, axis=-1, keepdims=True)
    return d * lax.rsqrt(v + EPS)


def _gelu(x):
    c0 = math.sqrt(2.0 / math.pi)
    u = x * (c0 + (c0 * 0.044715) * (x * x))
    hx = 0.5 * x
    return hx + hx * jnp.tanh(u)


def _pack(x):
    return pltpu.bitcast(x.astype(bf16), u32)


def _unpack(x):
    return pltpu.bitcast(x, bf16)


def _dot(a, b):
    return jnp.dot(a, b, preferred_element_type=f32)


class _Plan:
    def __init__(self, slots, nc, base):
        self.vpu = [tuple(hs for hs in range(HS) if (j, hs) in slots) for j in range(nc)]
        self.stream = [(j, hs) for j in range(nc) for hs in range(HS) if (j, hs) not in slots]
        self.first = {}
        for i, (j, _) in enumerate(self.stream):
            self.first.setdefault(j, i)
        self.groups = len(self.stream) // 2
        self.base = base


def _vpu_slots(n, nc, grp):
    per = nc // NL * HS
    quarters = []
    for t in range(NL):
        m = (n // 2 * (t + 1)) // NL * 2 - (n // 2 * t) // NL * 2
        quarters.append([divmod(t * per + int((i + t / NL) * per / m) * grp + y, HS)
                         for i in range(m // grp) for y in range(grp)])
    return quarters


def _thin(quarters, n):
    out = []
    for t, q in enumerate(quarters):
        m = (n // 2 * (t + 1)) // NL * 2 - (n // 2 * t) // NL * 2
        out += [q[(2 * i + 1) * len(q) // (2 * m)] for i in range(m)]
    return out


def _mxu_program(plan, order, blocks, weights, delta, lead):
    nc = len(order[0])
    total = len(blocks) * plan.groups
    n_dense = len(weights)
    span = total + len(blocks) * nc + n_dense * W_SLOTS / NL
    due = [(lead + sum(weights[:k])) * span / (lead + sum(weights)) for k in range(n_dense)]
    seqs = []
    for t in range(NL):
        dense = list(range(t, n_dense, NL))
        ops, issued, done = [], [], 0
        time = 0

        def scores():
            nonlocal time
            ub, g = divmod(len(issued), plan.groups)
            if ops and ops[-1][0] == 'scores' and ops[-1][2] == blocks[ub]:
                ops[-1] = ('scores', ops[-1][1] + 1, blocks[ub], ops[-1][3])
            else:
                ops.append(('scores', 1, blocks[ub], g))
            issued.append(time)
            time += 1

        def covered(slots):
            return len(issued) == total or (ops and ops[-1][1] >= slots)

        for b, u in enumerate(blocks):
            for step in range(nc):
                done += HS - len(plan.vpu[order[t][step]])
                last = (done + 1) // 2 - 1
                closing = b == len(blocks) - 1 and step == nc - 2
                if closing:
                    while len(issued) < total:
                        scores()
                while dense and (closing or (len(dense) > 1 and due[dense[0]] <= time)):
                    while not covered(4):
                        scores()
                    ops.append(('dense', W_SLOTS, dense.pop(0)))
                    time += W_SLOTS
                while len(issued) < total and (len(issued) <= last or time < issued[last] + delta
                                               or not covered(2)):
                    scores()
                ops.append(('values', 1, u, step))
                time += 1
        seqs.append(ops)
    free, merged = [0] * NL, []
    while any(seqs):
        t = min((t for t in range(NL) if seqs[t]), key=lambda t: free[t])
        op = seqs[t].pop(0)
        free[t] += op[1]
        merged.append((t,) + op)
    return merged


def _kernel(x_hbm, wq_hbm, wkt_hbm, wvt_hbm, wo_hbm, win_hbm, wsp_hbm, bsp_hbm, wout_hbm, c_hbm, wmod_hbm,
            out_hbm,
            x_v, wq_v, wkv_v, wo_v, win_v, wsp_v, bsp_v, wout_v, c_v, wmod_v,
            wqt_s, wo_s, win_s, h_s, k_s, kn_s, kb_s, vt_s, qt_s, qf_s, o_s, z2_s, mod_s,
            x1_s, z_s, g_s, h2_s, wt_s, ot_s, bias_s, zero_s, out_v, sems, wsems, osems,
            *, S, D, H, FH, TB, delta, lead, nv, nv0, merge, MB, nit, dev, wb, grp, dbg, NP):
    DH = D // H
    NC = S // T
    NQ = S // T
    NU = H // NL
    NX = S // TB
    ND = D // T
    NF = FH // T

    def cp(src, dst, i):
        return pltpu.make_async_copy(src, dst, sems.at[i])

    def tile_rows(i, n=T):
        return pl.ds(i * n if isinstance(i, int) else pl.multiple_of(i * n, n), n)

    c_cp = cp(c_hbm, c_v, 0)
    wmod_a = cp(wmod_hbm.at[:, pl.ds(0, 2 * D)], wmod_v.at[:, pl.ds(0, 2 * D)], 1)
    wq_cp = cp(wq_hbm, wq_v, 2)
    wk_cp = cp(wkt_hbm, wkv_v.at[pl.ds(0, DH), :], 3)
    wv_cp = cp(wvt_hbm, wkv_v.at[pl.ds(DH, DH), :], 4)
    wmod_b = cp(wmod_hbm.at[:, pl.ds(2 * D, 4 * D)], wmod_v.at[:, pl.ds(2 * D, 4 * D)], 5)
    wo_cp = cp(wo_hbm, wo_v, 6)
    win_cp = cp(win_hbm, win_v, 7)
    bsp_cp = cp(bsp_hbm, bsp_v, 8)
    wout_cp = cp(wout_hbm, wout_v, 9)
    x_cps = [cp(x_hbm.at[pl.ds(t * TB, TB), :], x_v.at[pl.ds(t * TB, TB), :], 10 + t) for t in range(NX)]

    NW = 4

    def wsp_cp(b):
        cols = tile_rows(b, S // NW)
        return pltpu.make_async_copy(wsp_hbm.at[:, cols], wsp_v.at[:, cols], wsems.at[b])

    for d in (c_cp, x_cps[0], wmod_a, wk_cp, wv_cp, wq_cp, *x_cps[1:]):
        d.start()

    key0 = lambda j, hs: j * T + (HS - 1 - hs) * 8
    quarters = _vpu_slots(nv, NC, grp)
    vidx = {s: i for i, s in enumerate(s for q in quarters for s in q)}
    plan = _Plan(set(vidx), NC, 0)
    plan0 = plan if nv0 == nv else _Plan(set(_thin(quarters, nv0)), NC, S // 2)
    order = [[(NC // NL * t + s) % NC for s in range(NC)] for t in range(NL)]

    zero_s[0] = 0

    def clear_gate():
        def clear(m, carry):
            g_s[tile_rows(m, 16), :] = jnp.zeros((16, FH), f32)
            return carry
        lax.fori_loop(0, S // 16, clear, 0)

    clear_gate()
    qscale = (DH ** -0.5) * math.log2(math.e)

    def project_kv(t):
        h = _unpack(h_s[t * TB // 2:(t + 1) * TB // 2, :])
        r = lax.dot_general(wkv_v[...], h, NT, preferred_element_type=f32)
        vt_s[:, t * TB:(t + 1) * TB] = _pack(r[DH:2 * DH])
        kt = jnp.concatenate([r[0:DH], jnp.zeros((T - DH, TB), f32)], axis=0).astype(bf16)
        kn = kt.T
        kn_s[t * TB // 2:(t + 1) * TB // 2, :] = pltpu.bitcast(kn, u32)
        kn = kn.astype(f32)
        mine = [(i, key0(j, hs) - t * TB) for (j, hs), i in vidx.items() if 0 <= key0(j, hs) - t * TB < TB]
        for d in range(DH):
            for i, r0 in mine:
                kb_s[i, d] = jnp.broadcast_to(kn[r0:r0 + 8, d:d + 1], (8, T))
        for p in ([plan] if plan0 is plan else [plan, plan0]):
            at = [a for a, (j, hs) in enumerate(p.stream) if 0 <= key0(j, hs) - t * TB < TB]
            rows = [kn[key0(*p.stream[a]) - t * TB:key0(*p.stream[a]) - t * TB + 8] for a in at]
            k_s[p.base + at[0] * 4:p.base + (at[-1] + 1) * 4, :] = _pack(jnp.concatenate(rows, axis=0))

    c_cp.wait()
    cf = c_v[...].astype(f32)
    sc = jnp.broadcast_to(cf * jax.nn.sigmoid(cf), (16, D)).astype(bf16)
    x_cps[0].wait()
    x1_s[0:TB, :] = _ln(x_v[0:TB, :].astype(f32))
    wmod_a.wait()
    mod_a = _dot(sc, wmod_v[:, 0:2 * D])[0:1]
    sa = mod_a[:, 0:D]
    ca1 = 1.0 + mod_a[:, D:2 * D]
    h_s[0:TB // 2, :] = _pack(x1_s[0:TB, :] * ca1 + sa)
    for d in (wk_cp, wv_cp, wq_cp):
        d.wait()
    wqt_s[...] = pltpu.bitcast(wq_v[...].T, u32)

    def rest_of_start_up():
        for t in range(1, NX):
            x_cps[t].wait()
            if t == NX - 1:
                for d in (wmod_b, wo_cp, win_cp, wsp_cp(0)):
                    d.start()
            project_kv(t - 1)
            h_s[t * TB // 2:(t + 1) * TB // 2, :] = _pack(_ln(x_v[t * TB:(t + 1) * TB, :].astype(f32)) * ca1 + sa)
        project_kv(NX - 1)

    held = []

    def accumulate(k, last, value):
        if k:
            value = value + held.pop()
        if k == last:
            return value
        held.append(value)
        return None

    def q_products(i, after=None, only=None):
        def product(r, k):
            hh = _unpack(h_s[tile_rows(i, T // 2), k * T:(k + 1) * T])
            w = _unpack(wqt_s[tile_rows(r, T // 2), k * T:(k + 1) * T])
            q = accumulate(k, ND - 1, lax.dot_general(w, hh, NT, preferred_element_type=f32))
            if q is not None:
                q = q * qscale
                qf_s[i % 2, tile_rows(r), :] = q
                qt_s[i % 2, tile_rows(r, T // 2), :] = _pack(q)
                if after is not None:
                    after(r, q)
        return [functools.partial(product, r, k) for r in (range(ND) if only is None else [only])
                for k in range(ND)]

    def mixer_products(i, split=False):
        rows = tile_rows(i)

        def norm_x1(part, parts):
            n = T // parts
            x1 = x1_s[pl.ds(pl.multiple_of((i + zero_s[0]) * T + part * n, n), n), :]
            h2_s[part * n // 2:(part + 1) * n // 2, :] = _pack(_ln(x1) * mod_s[2:3, :] + mod_s[1:2, :])

        def norm_z2(part, parts):
            n = T // parts
            z2 = z_s[pl.ds(pl.multiple_of(zero_s[0] * T + S + part * n, n), n), :]
            z2_s[part * n // 2:(part + 1) * n // 2, :] = _pack(_ln(z2))

        def out_proj(n, k):
            cols = slice(n * T, (n + 1) * T)
            if n == 0:
                o_s[:, k * T:(k + 1) * T] = pltpu.bitcast(ot_s[k * T:(k + 1) * T, :].astype(bf16).T, u32)
            a = _dot(_unpack(o_s[:, k * T:(k + 1) * T]), _unpack(wo_s[k * T // 2:(k + 1) * T // 2, cols]))
            a = accumulate(k, ND - 1, a)
            if a is not None:
                x1_s[rows, cols] = x_v[rows, cols].astype(f32) + mod_s[0:1, cols] * a
                if n == ND - 1:
                    norm_x1(0, ND if split else 1)

        def after_q(r, q):
            if split and r < ND - 1:
                x1_s[S:S + 8, 0:T] = q[0:8]
                norm_x1(r + 1, ND)

        def in_proj(n, k):
            z = _dot(_unpack(h2_s[:, k * T:(k + 1) * T]),
                     _unpack(win_s[k * T // 2:(k + 1) * T // 2, n * T:(n + 1) * T]))
            z = accumulate(k, ND - 1, z)
            if z is None:
                return
            if n < NF:
                z_s[rows, n * T:(n + 1) * T] = _gelu(z)
                if split and n < NF - 1:
                    norm_z2(n + 2, NF + 1)
            else:
                z_s[S:S + T, (n - NF) * T:(n - NF + 1) * T] = _gelu(z)
                if n == 2 * NF - 1:
                    if split:
                        norm_z2(0, NF + 1)
                        norm_z2(1, NF + 1)
                    else:
                        norm_z2(0, 1)
        return ([functools.partial(out_proj, n, k) for n in range(ND) for k in range(ND)],
                [functools.partial(in_proj, n, k) for n in (*range(NF, 2 * NF), *range(NF)) for k in range(ND)],
                after_q)

    def dense_products(i):
        out_proj, in_proj, after_q = mixer_products(i - 1, split=True)
        heavy = out_proj + q_products(jnp.minimum(i + 1, NQ - 1), after_q) + in_proj
        return [(p, wb) for p in heavy] + [(p, 1.0) for p in spatial_products(i - 1)]

    def stage_wsp(i, m):
        wt_s[m * T // 2:(m + 1) * T // 2, :] = pltpu.bitcast(wsp_v[m * T:(m + 1) * T, tile_rows(i)], u32)

    def spatial_products(i):
        def product(m, n):
            g_s[m * T:(m + 1) * T, n * T:(n + 1) * T] += _dot(
                _unpack(wt_s[m * T // 2:(m + 1) * T // 2, :]), _unpack(z2_s[:, n * T:(n + 1) * T]))
            if n == NF - 1:
                stage_wsp(i + 1, m)
        return [functools.partial(product, m, n) for m in range(NQ) for n in range(NF)]

    def setup():
        mod_b = _dot(sc, wmod_v[:, 2 * D:6 * D])[0:1]
        mod_s[0:1, :] = mod_b[:, 0:D]
        mod_s[1:2, :] = mod_b[:, D:2 * D]
        mod_s[2:3, :] = 1.0 + mod_b[:, 2 * D:3 * D]
        mod_s[3:4, :] = mod_b[:, 3 * D:4 * D]
        wo_s[...] = pltpu.bitcast(wo_v[...], u32)
        win_s[...] = pltpu.bitcast(win_v[...], u32)

    def attention(i, plan, blocks, dense, bad, head0=0):
        slot = i % 2
        st = {(u, t): dict(q=None, qf=None, acc=None, l=None) for u in blocks for t in range(NL)}
        probs = {}

        def finish(u, t, j, hs, s):
            e = jnp.exp2(s)
            z = st[u, t]
            z['l'] = e if z['l'] is None else z['l'] + e
            probs[u, t, j, hs] = e

        def vpu_scores(u, t, j, hs):
            z = st[u, t]
            if z['qf'] is None:
                z['qf'] = qf_s[slot, tile_rows(head0 + u * NL + t, DH), :]
            a = None
            for d in range(DH):
                term = kb_s[vidx[j, hs], d] * z['qf'][d:d + 1]
                a = term if a is None else a + term
            finish(u, t, j, hs, a)

        def mxu_scores(t, n, u, g0):
            z = st[u, t]
            if z['q'] is None:
                z['q'] = _unpack(jnp.concatenate([qt_s[slot, tile_rows(head0 + u * NL + t, DH // 2), :],
                                                  jnp.zeros(((T - DH) // 2, T), u32)], axis=0))
            gs = [(g + plan.first[order[t][0]] // 2) % plan.groups for g in range(g0, g0 + n)]
            cut = [a for a in range(1, n) if gs[a] != gs[a - 1] + 1]
            segs = [(gs[a], gs[b - 1] + 1) for a, b in zip([0] + cut, cut + [n])]
            lhs = jnp.concatenate([k_s[plan.base + a * 8:plan.base + b * 8, :] for a, b in segs], axis=0)
            s = _dot(_unpack(lhs), z['q'])
            for a, g in enumerate(gs):
                for y in range(2):
                    finish(u, t, *plan.stream[2 * g + y], s[(2 * a + y) * 8:(2 * a + y + 1) * 8])

        def values(t, u, step, bad):
            j = order[t][step]
            for hs in plan.vpu[j]:
                vpu_scores(u, t, j, hs)
            z = st[u, t]
            p = jnp.concatenate([probs.pop((u, t, j, hs)) for hs in reversed(range(HS))], axis=0)
            pv = _dot(_unpack(vt_s[:, j * T:(j + 1) * T]), p.astype(bf16))
            z['acc'] = pv if z['acc'] is None else pv + z['acc']
            if step == NC - 1:
                l = jnp.sum(z['l'], axis=0, keepdims=True)
                o = z['acc'] * (1.0 / l)
                ok = (l >= L_MIN) & (l <= L_MAX) & (jnp.abs(o) < jnp.inf)
                bad = jnp.where(ok, bad, 1.0)
                ot_s[tile_rows(head0 + u * NL + t, DH), :] = o
            return bad

        pending = list(dense)
        for t, kind, n, *args in _mxu_program(plan, order, blocks, [w for _, w in dense], delta, lead):
            if kind == 'dense':
                pending.pop(0)[0]()
            elif kind == 'scores':
                mxu_scores(t, n, *args)
            else:
                bad = values(t, *args, bad)
        return bad

    def run(products):
        for p in products:
            p()

    if dev:
        run(q_products(0))
        rest_of_start_up()
        for d in (wmod_b, wo_cp, win_cp, wsp_cp(0)):
            d.wait()
        setup()
        if 'W' in dbg:
            for b in range(1, NW):
                wsp_cp(b).start()
                wsp_cp(b).wait()
        def dev_body(i, bad):
            dense = dense_products(i)
            return attention(i, plan, range(dev[0]), dense[dev[1]:dev[2]], bad)
        out_v[0:DH, 0:T] = lax.fori_loop(1, nit or NQ, dev_body, jnp.zeros((DH, T), f32)).astype(bf16)
        d = pltpu.make_async_copy(out_v, out_hbm, osems.at[0])
        d.start()
        d.wait()
        return
    run(q_products(0))
    rest_of_start_up()
    bad = jnp.zeros((DH, T), f32)

    def first_tile(r, bad):
        return attention(0, plan0, range(NU // ND), [(p, 1.0) for p in q_products(1, only=r)], bad,
                         head0=r * (H // ND))

    if 'A' not in dbg:
        bad = lax.fori_loop(0, ND, first_tile, bad)
    for d in (wmod_b, wo_cp, win_cp):
        d.wait()
    for d in (*[wsp_cp(b) for b in range(1, NW)], bsp_cp, wout_cp):
        d.start()
    setup()

    def body(i, bad):
        @pl.when(i % (NQ // NW) == 0)
        def _():
            wsp_cp(i // (NQ // NW)).wait()

        dense = dense_products(i)
        if merge:
            return attention(i, plan, range(NU), dense, bad)
        run([p for p, _ in dense])
        return attention(i, plan, range(NU), [], bad)

    wsp_cp(0).wait()
    for m in range(NQ):
        stage_wsp(0, m)
    bad = lax.fori_loop(1, nit or NQ, body, bad)
    for b in range(((nit or NQ) - 1) // (NQ // NW) + 1, NW):
        wsp_cp(b).wait()

    @pl.when(jnp.max(bad) > (2.0 if 'A' in dbg else -1.0 if 'X' in dbg else 0.0))
    def _():
        if 'F' in dbg:
            g_s[0:8, 0:T] = jnp.zeros((8, T), f32)
            return
        clear_gate()

        def tile(i, carry):
            run(q_products(i))

            def head(hd, carry):
                q = _unpack(jnp.concatenate([qt_s[i % 2, tile_rows(hd, DH // 2), :],
                                             jnp.zeros(((T - DH) // 2, T), u32)], axis=0))
                s = _dot(_unpack(kn_s[...]), q)
                e = jnp.exp2(s - jnp.max(s, axis=0, keepdims=True))
                pv = _dot(_unpack(vt_s[...]), e.astype(bf16))
                ot_s[tile_rows(hd, DH), :] = pv * (1.0 / jnp.sum(e, axis=0, keepdims=True))
                return carry
            lax.fori_loop(0, H, head, 0)

            @pl.when(i < NQ - 1)
            def _():
                for products in mixer_products(i)[:2]:
                    run(products)

                def rows(m, carry):
                    g_s[tile_rows(m), :] += _dot(wsp_v[tile_rows(m), tile_rows(i)], _unpack(z2_s[...]))
                    return carry
                lax.fori_loop(0, NQ, rows, 0)
            return carry
        lax.fori_loop(0, NQ, tile, 0)

    bsp_cp.wait()
    wout_cp.wait()
    for products in mixer_products(NQ - 1)[:2]:
        run(products)
    gb = mod_s[3:4, :]
    bt = bsp_v[...].astype(f32).T
    NM = S // MB // NP

    def out_cp(m):
        return pltpu.make_async_copy(out_v.at[tile_rows(m, MB), :], out_hbm.at[tile_rows(m, MB), :], osems.at[m])

    for j in range(NQ):
        bias_s[j] = jnp.broadcast_to(bt[:, j:j + 1], (T, T))

    def gate(part, carry):
        for a in range(NM):
            m = part * NM + a
            rows = tile_rows(m, MB)
            bias = jnp.concatenate([bias_s[m * (MB // T) + j] for j in range(MB // T)], axis=0)
            g = _dot(_unpack(wt_s[tile_rows(m, MB // 2), :]), _unpack(z2_s[...]))
            g = g + (g_s[rows, :] + jnp.concatenate([bias] * NF, axis=1))
            y = _dot((z_s[rows, :] * g).astype(bf16), wout_v[...])
            out_v[rows, :] = (x1_s[rows, :] + gb * y).astype(bf16)
            out_cp(m).start()
        return carry

    if NP == 1:
        gate(0, 0)
    else:
        lax.fori_loop(0, NP, gate, 0)
    for m in range(S // MB):
        out_cp(m).wait()


def make(TB=512, delta=11, lead=1.0, nv=46, nv0=36, merge=True, MB=256, nit=0, dev=None, wb=0.8, grp=1, dbg='', NP=2, flags=None):
    def fn(A_x, A_wq, A_wk, A_wv, A_wo, B_x, B_w_in, B_w_sp, B_b_sp, B_w_out, c, w_mod):
        B, S, D = A_x.shape
        H = 32
        DH = D // H
        FH = B_w_out.shape[0]
        V = pltpu.VMEM
        dma = pltpu.SemaphoreType.DMA
        scratch = [
            V((S, D), bf16), V((D, D), bf16), V((2 * DH, D), bf16), V((D, D), bf16), V((D, 2 * FH), bf16),
            V((S, S), bf16), V((S // T, T), bf16), V((FH, D), bf16), V((1, D), bf16), V((D, 6 * D), bf16),
            V((D // 2, D), u32), V((D // 2, D), u32), V((D // 2, 2 * FH), u32), V((S // 2, D), u32),
            V((S, T), u32), V((S // 2, T), u32), V((nv, DH, 8, T), f32), V((DH // 2, S), u32),
            V((2, D // 2, T), u32), V((2, D, T), f32), V((T // 2, D), u32), V((T // 2, FH), u32), V((8, D), f32),
            V((S + 8, D), f32), V((S + T, FH), f32), V((S, FH), f32), V((T // 2, D), u32),
            V((S // 2, T), u32), V((D, T), f32), V((S // T, T, T), f32), pltpu.SMEM((1,), jnp.int32), V((S, D), bf16),
            dma((10 + S // TB,)), dma((4,)), dma((S // MB,)),
        ]
        out = pl.pallas_call(
            functools.partial(_kernel, S=S, D=D, H=H, FH=FH, TB=TB, delta=delta, lead=lead, nv=nv, nv0=nv0,
                              merge=merge, MB=MB, nit=nit, dev=dev, wb=wb, grp=grp, dbg=dbg, NP=NP),
            out_shape=jax.ShapeDtypeStruct((S, D), A_x.dtype),
            in_specs=[pl.BlockSpec(memory_space=pl.ANY)] * 11,
            out_specs=pl.BlockSpec(memory_space=pl.ANY),
            scratch_shapes=scratch,
            compiler_params=pltpu.CompilerParams(vmem_limit_bytes=100 * 2**20, flags=flags),
            name='fused',
        )(A_x.reshape(S, D), A_wq, A_wk.T, A_wv.T, A_wo, B_w_in, B_w_sp, B_b_sp.reshape(S // T, T), B_w_out, c, w_mod)
        return out.reshape(B, S, D)
    return fn


@jax.jit
def pallas_adaLN_cond__grouped_kv_mqa__mixer_gmlp__prompt_kernel(
    A_x: jax.Array,
    A_wq: jax.Array,
    A_wk: jax.Array,
    A_wv: jax.Array,
    A_wo: jax.Array,
    B_x: jax.Array,
    B_w_in: jax.Array,
    B_w_sp: jax.Array,
    B_b_sp: jax.Array,
    B_w_out: jax.Array,
    c: jax.Array,
    w_mod: jax.Array,
):
    return make()(A_x, A_wq, A_wk, A_wv, A_wo, B_x, B_w_in, B_w_sp, B_b_sp, B_w_out, c, w_mod)
```

```python
import functools
import math

import jax
import jax.numpy as jnp
from jax import lax
import jax.experimental.pallas as pl
import jax.experimental.pallas.tpu as pltpu

f32, bf16, u32 = jnp.float32, jnp.bfloat16, jnp.uint32

HEADS = 32
EPS = 1e-5
T = 128
NL = 4
HS = T // 8
W_SLOTS = T // 16
NX = 4
L_MIN, L_MAX = 2.0 ** -40, 2.0 ** 80

VPU_SLOTS_MIXED = 52
VPU_SLOTS_PLAIN = 42
PLAIN_HEADS = 11
EARLY_SPATIAL = 8
VALUE_DELAY = 10
MIN_RUN = 4
STAGGER = 2
DENSE_GAP = 0.7
FIRST_SPLIT = 24


def _pack(x):
    if x.shape[1] != T:
        return pltpu.bitcast(x.astype(bf16), u32)
    h = x.shape[0] // 2
    if h % 16:
        return _pack(jnp.concatenate([x, x], axis=1))[:, :T]
    y = _pack(jnp.concatenate([x[:h], x[h:]], axis=1))
    return jnp.concatenate([y[:, :T], y[:, T:]], axis=0)


def _unpack(x):
    return pltpu.bitcast(x, bf16)


def _dot(a, b):
    return jnp.dot(a, b, preferred_element_type=f32)


def _dot_nt(a, b):
    return lax.dot_general(a, b, (((1,), (1,)), ((), ())), preferred_element_type=f32)


def _gelu_of_half(hx):
    c0 = 2.0 * math.sqrt(2.0 / math.pi)
    return hx + hx * jnp.tanh(hx * (c0 + (4.0 * 0.044715 * c0) * (hx * hx)))


class _Moments:
    def __init__(self):
        self.n = 0

    def add(self, x):
        for r in range(0, x.shape[0], 8):
            v = x[r:r + 8]
            if self.n == 0:
                self.pivot = v
            else:
                d = v - self.pivot
                self.s1 = d if self.n == 1 else self.s1 + d
                self.s2 = d * d if self.n == 1 else self.s2 + d * d
            self.n += 1

    def mean_rstd(self):
        off = self.s1 * (1.0 / self.n)
        part = self.pivot + off
        mean = jnp.sum(part, axis=0, keepdims=True) * 0.125
        d = part - mean
        m2 = (self.s2 * (1.0 / self.n) - off * off) + d * d
        var = jnp.maximum(jnp.sum(m2, axis=0, keepdims=True) * 0.125, 0.0)
        return mean, lax.rsqrt(var + EPS)


def _per_quarter(n, c):
    return (n // 2 * (c + 1)) // NL * 2 - (n // 2 * c) // NL * 2


def _vpu_slots(n, tiles):
    per = tiles // NL * HS
    return [[divmod(c * per + int((i + c / NL) * per / _per_quarter(n, c)), HS)
             for i in range(_per_quarter(n, c))] for c in range(NL)]


def _thin(quarters, n):
    return [[q[(2 * i + 1) * len(q) // (2 * _per_quarter(n, c))] for i in range(_per_quarter(n, c))]
            for c, q in enumerate(quarters)]


class _Plan:
    def __init__(self, quarters, tiles, base):
        self.per = tiles // NL
        picked = [s for q in quarters for s in q]
        self.vpu = [tuple(hs for hs in range(HS) if (j, hs) in picked) for j in range(tiles)]
        self.stream = [[(j, hs) for j in range(c * self.per, (c + 1) * self.per) for hs in range(HS)
                        if (j, hs) not in picked] for c in range(NL)]
        self.groups = [len(s) // 2 for s in self.stream]
        self.first = [base + 8 * sum(self.groups[:c]) for c in range(NL)]


def _mxu_program(plans, n_dense, first):
    heads, per = len(plans), plans[0].per
    todo = [[(u, g) for u in range(heads) for g in range(plans[u].groups[(t + u) % NL])] for t in range(NL)]
    span = len(todo[0]) + heads * per + n_dense * W_SLOTS / NL
    start = sum(u < first for u, _ in todo[0]) + first * per
    due = [start + k * (span - start) / max(n_dense, 1) for k in range(n_dense + 1)]
    seqs = [[] for _ in range(NL)]
    issued = [[] for _ in range(NL)]
    time, done, taken, steps = [0] * NL, [0] * NL, [0] * NL, [0] * NL
    started, last_start = 0, -span

    def scores(t):
        u, g = todo[t][len(issued[t])]
        if seqs[t] and seqs[t][-1][0] == 'scores' and seqs[t][-1][2] == u:
            seqs[t][-1] = ('scores', seqs[t][-1][1] + 1, u, seqs[t][-1][3])
        else:
            seqs[t].append(('scores', 1, u, g))
        issued[t].append(time[t])
        time[t] += 1

    def covered(t, slots):
        return len(issued[t]) == len(todo[t]) or (seqs[t] and seqs[t][-1][1] >= slots)

    while min(steps) < heads * per:
        t = min((t for t in range(NL) if steps[t] < heads * per), key=lambda t: time[t])
        u, step = divmod(steps[t], per)
        done[t] += HS - len(plans[u].vpu[(t + u) % NL * per + step])
        last = (done[t] + 1) // 2 - 1
        closing = steps[t] == heads * per - 2
        while closing and len(issued[t]) < len(todo[t]):
            scores(t)
        while taken[t] < n_dense // NL:
            now = (taken[t] <= min(taken) + 1 and due[started] <= time[t] + MIN_RUN
                   and time[t] + MIN_RUN >= last_start + DENSE_GAP * (due[started + 1] - due[started]))
            if not (closing or (now and taken[t] < n_dense // NL - 1 and steps[t] > 0)):
                break
            while not covered(t, MIN_RUN):
                scores(t)
            seqs[t].append(('dense', W_SLOTS))
            last_start = time[t]
            time[t] += W_SLOTS
            taken[t] += 1
            started += 1
            if not closing:
                break
        wait = VALUE_DELAY + (STAGGER * t if steps[t] == 0 else 0)
        while len(issued[t]) < len(todo[t]) and (len(issued[t]) <= last or time[t] < issued[t][last] + wait
                                                 or not covered(t, 2)):
            scores(t)
        seqs[t].append(('values', 1, u, step))
        time[t] += 1
        steps[t] += 1
    assert started == n_dense
    free, merged = [0] * NL, []
    while any(seqs):
        t = min((t for t in range(NL) if seqs[t]), key=lambda t: free[t])
        op = seqs[t].pop(0)
        free[t] += op[1]
        merged.append((t,) + op)
    return merged


def _kernel(x_hbm, wq_hbm, wkt_hbm, wvt_hbm, wo_hbm, win_hbm, wsp_hbm, bsp_hbm, wout_hbm, c_hbm, wmod_hbm,
            out_hbm,
            x_v, wq_v, wkv_v, wo_v, win_v, wsp_v, bsp_v, wout_v, wmod_v,
            wq_s, wo_s, win_s, wout_s, wt_s, mod_s, row_s, h_s, kv_s, k_s, kn_s, kb_s, vt_s, qt_s, qf_s,
            o_s, h2_s, z2_s, bad_s, x1c_s, z2f_s, x1_s, z_s, g_s, out_v, c_v, zero_s, sems, wsems, osems):
    S, D = x_hbm.shape
    FH = wout_hbm.shape[0]
    H = HEADS
    DH = D // H
    NQ = S // T
    ND, NF = D // T, FH // T
    XT = NQ // NX

    def tile(i, n=T):
        return pl.ds(i * n if isinstance(i, int) else pl.multiple_of(i * n, n), n)

    def half(i):
        return tile(i, T // 2)

    def cp(src, dst, i):
        return pltpu.make_async_copy(src, dst, sems.at[i])

    c_cp = cp(c_hbm, c_v, 0)
    wmod_a = cp(wmod_hbm.at[:, pl.ds(0, 2 * D)], wmod_v.at[:, pl.ds(0, 2 * D)], 1)
    wq_cp = cp(wq_hbm, wq_v, 2)
    wk_cp = cp(wkt_hbm, wkv_v.at[pl.ds(0, DH), :], 3)
    wv_cp = cp(wvt_hbm, wkv_v.at[pl.ds(DH, DH), :], 4)
    wmod_b = cp(wmod_hbm.at[:, pl.ds(2 * D, 4 * D)], wmod_v.at[:, pl.ds(2 * D, 4 * D)], 5)
    wo_cp = cp(wo_hbm, wo_v.at[pl.ds(0, D), :], 6)
    win_cp = cp(win_hbm, win_v.at[pl.ds(0, D), :], 7)
    bsp_cp = cp(bsp_hbm, bsp_v, 8)
    wout_cp = cp(wout_hbm, wout_v, 9)

    def x_cp(b):
        return cp(x_hbm.at[tile(b, XT * T), :], x_v.at[tile(b, XT * T), pl.ds(0, D)], 10 + b)

    def wsp_cp(b):
        return pltpu.make_async_copy(wsp_hbm.at[:, tile(b, XT * T)], wsp_v.at[:, tile(b, XT * T)], wsems.at[b])

    def out_cp(m):
        return pltpu.make_async_copy(out_v.at[tile(m), :], out_hbm.at[tile(m), :], osems.at[m])

    for d in (c_cp, x_cp(0), wmod_a, wk_cp, wv_cp, *[x_cp(b) for b in range(1, NX)], wq_cp):
        d.start()

    def key0(j, hs):
        return j * T + (HS - 1 - hs) * 8

    quarters = _vpu_slots(VPU_SLOTS_MIXED, NQ)
    vidx = {s: i for i, s in enumerate(s for q in quarters for s in q)}
    mixed = _Plan(quarters, NQ, 0)
    plain = _Plan(_thin(quarters, VPU_SLOTS_PLAIN), NQ, S // 2)

    zero_s[0] = 0

    def fence(ref, value):
        ref[pl.ds(pl.multiple_of(ref.shape[0] - 8 + zero_s[0] * 8, 8), 8), 0:T] = value

    def stage(ref, k, value):
        ref[half(k), :] = value
        fence(ref, jnp.zeros((8, T), ref.dtype))

    def clear_gate():
        def clear(m, carry):
            g_s[m] = jnp.zeros((FH, T), f32)
            return carry
        lax.fori_loop(0, NQ, clear, 0)

    def normalise_x(b):
        x = x_v[tile(b, XT * T), 0:D].astype(f32)
        d = x - jnp.mean(x, axis=1, keepdims=True)
        return d * lax.rsqrt(jnp.mean(d * d, axis=1, keepdims=True) + EPS)

    def project_kv(b):
        kv_s[:, tile(b, XT * T)] = _dot_nt(wkv_v[...], _unpack(h_s[tile(b, XT * T // 2), :]))

    def arrange_keys():
        r = kv_s[...]
        vt_s[...] = _pack(r[DH:2 * DH])
        kn = jnp.concatenate([r[0:DH], jnp.zeros((T - DH, S), f32)], axis=0).astype(bf16).T
        kn_s[...] = pltpu.bitcast(kn, u32)
        kn = kn.astype(f32)

        def keys(slots):
            return jnp.concatenate([kn[key0(*slot):key0(*slot) + 8] for slot in slots], axis=0)

        for p in (mixed, plain):
            k_s[p.first[0]:p.first[0] + 8 * sum(p.groups), :] = pltpu.bitcast(
                keys([s for c in p.stream for s in c]).astype(bf16), u32)
        picked = keys(vidx)
        nm = DH // 2
        pick = (lax.broadcasted_iota(jnp.int32, (DH, nm * T), 0)
                == lax.broadcasted_iota(jnp.int32, (DH, nm * T), 1) // T).astype(f32)
        pick = jnp.concatenate([pick, jnp.zeros((T - DH, nm * T), f32)], axis=0).astype(bf16)
        wide = _dot(picked.astype(bf16), pick)
        for d in range(DH):
            for i in range(len(vidx)):
                rows = slice(8 * i, 8 * i + 8)
                kb_s[i, d] = (wide[rows, d * T:(d + 1) * T] if d < nm
                              else jnp.broadcast_to(picked[rows, d:d + 1], (8, T)))

    clear_gate()
    c_cp.wait()
    cf = c_v[...].astype(f32)
    sc = jnp.broadcast_to(cf * jax.nn.sigmoid(cf), (16, D)).astype(bf16)
    x_cp(0).wait()
    xn = normalise_x(0)
    wmod_a.wait()
    mod_a = _dot(sc, wmod_v[:, 0:2 * D])[0:1]
    shift, scale = mod_a[:, 0:D], 1.0 + mod_a[:, D:2 * D]
    h_s[tile(0, XT * T // 2), :] = _pack(xn * scale + shift)

    held, staging = [], []

    def accumulate(k, value):
        if k:
            value = value + held.pop()
        if k < ND - 1:
            held.append(value)
            return None
        if staging:
            staging.pop(0)(value)
        return value

    def query_products(i):
        def product(r, k):
            q = accumulate(k, _dot_nt(_unpack(wq_s[half(r), tile(k)]), _unpack(h_s[half(i), tile(k)])))
            if q is not None:
                q = q * ((DH ** -0.5) * math.log2(math.e))
                qt_s[half(r), :] = _pack(q)
                qf_s[tile(r), :] = q
        return [functools.partial(product, r, k) for r in range(ND) for k in range(ND)]

    def mixer_products(i):
        x1m, z2m, x1_stats, z2_stats = _Moments(), _Moments(), [], []

        def out_proj(n, k):
            a = accumulate(k, _dot(_unpack(wo_s[half(n), tile(k)]), _unpack(o_s[half(k), :])))
            if a is not None:
                x1 = x_v[tile(i), tile(n)].T.astype(f32) + mod_s[0, tile(n), :] * a
                x1c_s[tile(n), :] = x1
                x1_s[i, tile(n), :] = x1
                x1m.add(x1)
                if n == ND - 1:
                    x1_stats.extend(x1m.mean_rstd())

        def normalise_z2(n):
            stage(z2_s, n, _pack((z2f_s[tile(n), :] - z2_stats[0]) * z2_stats[1]))

        def in_proj(n, k):
            if n == NF:
                mean, rstd = x1_stats
                stage(h2_s, k, _pack((x1c_s[tile(k), :] - mean) * rstd * mod_s[2, tile(k), :]
                                     + mod_s[1, tile(k), :]))
            z = accumulate(k, _dot(_unpack(win_s[half(n), tile(k)]), _unpack(h2_s[half(k), :])))
            if z is None:
                return
            z = _gelu_of_half(z)
            if n < NF:
                z_s[i, tile(n), :] = z
                if n < NF - 1:
                    fence(z2f_s, z[0:8])
                    normalise_z2(n + 1)
            else:
                z2f_s[tile(n - NF), :] = z
                z2m.add(z)
                if n == 2 * NF - 1:
                    z2_stats.extend(z2m.mean_rstd())
                    normalise_z2(0)
        return ([functools.partial(out_proj, n, k) for n in range(ND) for k in range(ND)],
                [functools.partial(in_proj, n, k) for n in (*range(NF, 2 * NF), *range(NF)) for k in range(ND)])

    def stage_wsp(i, m, token):
        wsp_v[0:16, pl.ds(pl.multiple_of(S + zero_s[0] * T, T), T)] = token[0:16].astype(bf16)
        wt_s[half(m), :] = pltpu.bitcast(wsp_v[tile(m), tile(i)].T, u32)
        if m == NQ - 1:
            fence(wt_s, jnp.zeros((8, T), u32))

    def spatial_products():
        def product(m, n):
            g_s[m, tile(n), :] += _dot(_unpack(z2_s[half(n), :]), _unpack(wt_s[half(m), :]))
        return [functools.partial(product, m, n) for m in range(NQ) for n in range(NF)]

    def run(products):
        for p in products:
            p()

    def padded_query(hd):
        return _unpack(jnp.concatenate([qt_s[tile(hd, DH // 2), :], jnp.zeros(((T - DH) // 2, T), u32)], axis=0))

    def attention(plans, dense=(), first=0, head0=0, side=()):
        dense, side = list(dense), list(side)
        n_side = 1.3 * len(side)
        q, rows, sums, accs, probs, closed = {}, {}, {}, {}, {}, {}

        def keep(u, t, slot, e):
            sums[u, t] = e if (u, t) not in sums else sums[u, t] + e
            probs[u, slot] = e

        def vpu_scores(u, t, slot):
            if u not in rows:
                qf = qf_s[tile(head0 + u + zero_s[0], DH), :]
                rows[u] = [jnp.broadcast_to(qf[d:d + 1], (8, T)) for d in range(DH)]
            part = [None, None]
            for d in range(DH):
                term = kb_s[vidx[slot], d] * rows[u][d]
                part[d % 2] = term if d < 2 else part[d % 2] + term
            keep(u, t, slot, jnp.exp2(part[0] + part[1]))

        def mxu_scores(t, n, u, g0):
            if u not in q:
                q[u] = padded_query(head0 + u)
            plan, c = plans[u], (t + u) % NL
            e = jnp.exp2(_dot(_unpack(k_s[plan.first[c] + 8 * g0:plan.first[c] + 8 * (g0 + n), :]), q[u]))
            for a in range(2 * n):
                keep(u, t, plan.stream[c][2 * g0 + a], e[a * 8:(a + 1) * 8])

        def values(t, u, step):
            plan = plans[u]
            j = (t + u) % NL * plan.per + step
            for hs in plan.vpu[j]:
                vpu_scores(u, t, (j, hs))
            p = jnp.concatenate([probs.pop((u, (j, hs))) for hs in reversed(range(HS))], axis=0)
            pv = _dot(_unpack(vt_s[:, tile(j)]), p.astype(bf16))
            accs[u] = pv if u not in accs else pv + accs[u]
            if side and t == 0 and (len(side) + 1) * len(plans) * plan.per > n_side * (
                    (len(plans) - u) * plan.per - step):
                side.pop(0)(pv)
            closed[u] = closed.get(u, 0) + 1
            if closed[u] == NQ:
                l = functools.reduce(lambda a, b: a + b, [sums.pop((u, c)) for c in range(NL)])
                l = jnp.sum(l, axis=0, keepdims=True)
                o = accs.pop(u) * (1.0 / l)
                size = jnp.abs(o)
                ok = (l >= L_MIN) & (l <= L_MAX) & (size[0:8] < jnp.inf) & (size[8:16] < jnp.inf)
                bad_s[...] = jnp.where(ok, bad_s[...], 1.0)
                o_s[tile(head0 + u, DH // 2), :] = _pack(o)

        for t, kind, n, *args in _mxu_program(plans, len(dense), first):
            if kind == 'dense':
                dense.pop(0)()
            elif kind == 'scores':
                mxu_scores(t, n, *args)
            else:
                values(t, *args)
        assert not side and not probs

    def normalise_block(b, carry):
        x_cp(b).wait()
        project_kv(b - 1)
        h_s[tile(b, XT * T // 2), :] = _pack(normalise_x(b) * scale + shift)
        return carry

    wk_cp.wait()
    wv_cp.wait()
    lax.fori_loop(1, NX, normalise_block, 0)
    for d in (wmod_b, wo_cp, win_cp):
        d.start()
    wq_cp.wait()
    wq_s[...] = pltpu.bitcast(wq_v[...].T, u32)
    project_kv(NX - 1)
    arrange_keys()
    run(query_products(0))
    bad_s[...] = jnp.zeros((8, T), f32)
    attention([plain] * FIRST_SPLIT)

    for d in (*[wsp_cp(b) for b in range(NX)], bsp_cp, wout_cp):
        d.start()
    for d in (wmod_b, wo_cp, win_cp):
        d.wait()
    mod_b = _dot(sc, wmod_v[:, 2 * D:6 * D])[0:1]
    row_s[0:1, :] = mod_b[:, 0:D]
    row_s[1:2, :] = 0.5 * mod_b[:, D:2 * D]
    row_s[2:3, :] = 0.5 * (1.0 + mod_b[:, 2 * D:3 * D])
    row_s[3:4, :] = mod_b[:, 3 * D:4 * D]

    def spread_row(v, token):
        fence(row_s, token[0:8])
        row = row_s[v:v + 1, :]
        for n in range(ND):
            mod_s[v, tile(n), :] = jnp.broadcast_to(row[:, n * T:(n + 1) * T], (T, T)).T

    def transpose(src, dst, n, token):
        src[pl.ds(pl.multiple_of(D + zero_s[0] * 16, 16), 16), 0:T] = token.astype(bf16)
        dst[half(n), :] = pltpu.bitcast(src[0:D, tile(n)].T, u32)

    attention([plain] * (H - FIRST_SPLIT), head0=FIRST_SPLIT,
              side=[functools.partial(spread_row, v) for v in range(4)]
              + [functools.partial(transpose, wo_v, wo_s, n) for n in range(ND)]
              + [functools.partial(transpose, win_v, win_s, n) for n in range(2 * NF)])

    def body(i, carry):
        @pl.when((i - 1) % XT == 0)
        def _():
            wsp_cp((i - 1) // XT).wait()

        out_proj, in_proj = mixer_products(i - 1)
        staging.extend(functools.partial(stage_wsp, i - 1, m) for m in range(NQ))
        run(out_proj + query_products(i) + in_proj)
        spatial = spatial_products()
        run(spatial[:EARLY_SPATIAL])
        attention([plain] * PLAIN_HEADS + [mixed] * (H - PLAIN_HEADS), spatial[EARLY_SPATIAL:], first=PLAIN_HEADS)
        return carry

    lax.fori_loop(1, NQ, body, 0)

    @pl.when(jnp.max(bad_s[...]) > 0.0)
    def _():
        clear_gate()

        def redo(i, carry):
            run(query_products(i))

            def head(hd, carry):
                s = _dot(_unpack(kn_s[...]), padded_query(hd))
                e = jnp.exp2(s - jnp.max(s, axis=0, keepdims=True))
                pv = _dot(_unpack(vt_s[...]), e.astype(bf16))
                o_s[tile(hd, DH // 2), :] = _pack(pv * (1.0 / jnp.sum(e, axis=0, keepdims=True)))
                return carry
            lax.fori_loop(0, H, head, 0)

            @pl.when(i < NQ - 1)
            def _():
                out_proj, in_proj = mixer_products(i)
                run(out_proj + in_proj)

                def spatial(m, carry):
                    g_s[m] += _dot_nt(_unpack(z2_s[0:FH // 2, :]), wsp_v[tile(m), tile(i)])
                    return carry
                lax.fori_loop(0, NQ, spatial, 0)
            return carry
        lax.fori_loop(0, NQ, redo, 0)

    bsp_cp.wait()
    wout_cp.wait()
    wout_s[...] = pltpu.bitcast(wout_v[...].T, u32)
    out_proj, in_proj = mixer_products(NQ - 1)
    staging.extend(functools.partial(stage_wsp, NQ - 1, m) for m in range(NQ))
    run(out_proj + in_proj)
    bias = bsp_v[...].astype(f32)
    for m in range(NQ):
        qf_s[tile(m, 8), :] = jnp.broadcast_to(bias[m:m + 1], (8, T))

    def gate(part, carry):
        for a in range(2):
            ms = [(part * 2 + a) * XT + j for j in range(XT)]
            g = _dot(_unpack(z2_s[0:FH // 2, :]), jnp.concatenate([_unpack(wt_s[half(m), :]) for m in ms], axis=1))
            u = []
            for j, m in enumerate(ms):
                prior = g_s[m].reshape(FH // 8, 8, T) + qf_s[tile(m, 8), :][None]
                u.append((z_s[m] * (g[:, j * T:(j + 1) * T] + prior.reshape(FH, T))).astype(bf16))
            y = _dot(_unpack(wout_s[...]), jnp.concatenate(u, axis=1))
            for j, m in enumerate(ms):
                out_v[tile(m), :] = (x1_s[m] + mod_s[3] * y[:, j * T:(j + 1) * T]).astype(bf16).T
                out_cp(m).start()
        return carry

    lax.fori_loop(0, NX // 2, gate, 0)
    for m in range(NQ):
        out_cp(m).wait()


@jax.jit
def pallas_adaLN_cond__grouped_kv_mqa__mixer_gmlp__prompt_kernel(
    A_x: jax.Array,
    A_wq: jax.Array,
    A_wk: jax.Array,
    A_wv: jax.Array,
    A_wo: jax.Array,
    B_x: jax.Array,
    B_w_in: jax.Array,
    B_w_sp: jax.Array,
    B_b_sp: jax.Array,
    B_w_out: jax.Array,
    c: jax.Array,
    w_mod: jax.Array,
):
    del B_x
    B, S, D = A_x.shape
    DH = D // HEADS
    FH = B_w_out.shape[0]
    NQ = S // T
    V = pltpu.VMEM
    dma = pltpu.SemaphoreType.DMA
    scratch = [
        V((S, D + T), bf16), V((D, D), bf16), V((2 * DH, D), bf16), V((D + 16, D), bf16),
        V((D + 16, 2 * FH), bf16), V((S, S + T), bf16), V((NQ, T), bf16), V((FH, D), bf16), V((D, 6 * D), bf16),
        V((D // 2, D), u32), V((D // 2, D), u32), V((FH, D), u32), V((D // 2, FH), u32), V((S // 2 + 8, T), u32),
        V((4, D, T), f32), V((16, D), f32), V((S // 2, D), u32), V((2 * DH, S), f32),
        V((S, T), u32), V((S // 2, T), u32), V((VPU_SLOTS_MIXED, DH, 8, T), f32), V((DH // 2, S), u32),
        V((D // 2, T), u32), V((D, T), f32),
        V((D // 2, T), u32), V((D // 2 + 8, T), u32), V((FH // 2 + 8, T), u32),
        V((8, T), f32), V((D, T), f32), V((FH + 8, T), f32),
        V((NQ, D, T), f32), V((NQ, FH, T), f32), V((NQ, FH, T), f32), V((S, D), bf16),
        V((1, D), bf16), pltpu.SMEM((1,), jnp.int32),
        dma((10 + NX,)), dma((NX,)), dma((NQ,)),
    ]
    out = pl.pallas_call(
        _kernel,
        out_shape=jax.ShapeDtypeStruct((S, D), A_x.dtype),
        in_specs=[pl.BlockSpec(memory_space=pl.ANY)] * 11,
        out_specs=pl.BlockSpec(memory_space=pl.ANY),
        scratch_shapes=scratch,
        compiler_params=pltpu.CompilerParams(
            vmem_limit_bytes=100 * 2**20, flags={'XLA_TPU_EVENLY_DISTRIBUTE_CRITICAL_NODES': True}),
        name='fused',
    )(A_x.reshape(S, D), A_wq, A_wk.T, A_wv.T, A_wo, B_w_in, B_w_sp, B_b_sp.reshape(NQ, T), B_w_out, c, w_mod)
    return out.reshape(B, S, D)
```

```python
import functools
import math

import jax
import jax.numpy as jnp
from jax import lax
import jax.experimental.pallas as pl
import jax.experimental.pallas.tpu as pltpu

f32, bf16, u32 = jnp.float32, jnp.bfloat16, jnp.uint32

HEADS = 32
EPS = 1e-5
T = 128
NL = 4
HS = T // 8
W_SLOTS = T // 16
NX = 4
L_MIN, L_MAX = 2.0 ** -40, 2.0 ** 80

VPU_SLOTS_MIXED = 52
VPU_SLOTS_PLAIN = 42
PLAIN_HEADS = 11
EARLY_SPATIAL = 8
VALUE_DELAY = 10
MIN_RUN = 4
STAGGER = 2
DENSE_GAP = 0.7
LATE_TILES = 3
FIRST_SPLIT = 24


def _pack(x):
    if x.shape[1] != T:
        return pltpu.bitcast(x.astype(bf16), u32)
    h = x.shape[0] // 2
    if h % 16:
        return _pack(jnp.concatenate([x, x], axis=1))[:, :T]
    y = _pack(jnp.concatenate([x[:h], x[h:]], axis=1))
    return jnp.concatenate([y[:, :T], y[:, T:]], axis=0)


def _unpack(x):
    return pltpu.bitcast(x, bf16)


def _dot(a, b):
    return jnp.dot(a, b, preferred_element_type=f32)


def _dot_nt(a, b):
    return lax.dot_general(a, b, (((1,), (1,)), ((), ())), preferred_element_type=f32)


def _gelu_of_half(hx):
    c0 = 2.0 * math.sqrt(2.0 / math.pi)
    return hx + hx * jnp.tanh(hx * (c0 + (4.0 * 0.044715 * c0) * (hx * hx)))


class _Moments:
    def __init__(self):
        self.n = 0

    def add(self, x):
        for r in range(0, x.shape[0], 8):
            v = x[r:r + 8]
            if self.n == 0:
                self.pivot = v
            else:
                d = v - self.pivot
                self.s1 = d if self.n == 1 else self.s1 + d
                self.s2 = d * d if self.n == 1 else self.s2 + d * d
            self.n += 1

    def mean_rstd(self):
        off = self.s1 * (1.0 / self.n)
        part = self.pivot + off
        mean = jnp.sum(part, axis=0, keepdims=True) * 0.125
        d = part - mean
        m2 = (self.s2 * (1.0 / self.n) - off * off) + d * d
        var = jnp.maximum(jnp.sum(m2, axis=0, keepdims=True) * 0.125, 0.0)
        return mean, lax.rsqrt(var + EPS)


def _per_quarter(n, c):
    return (n // 2 * (c + 1)) // NL * 2 - (n // 2 * c) // NL * 2


def _vpu_slots(n, tiles):
    per = tiles // NL * HS
    return [[divmod(c * per + int((i + c / NL) * per / _per_quarter(n, c)), HS)
             for i in range(_per_quarter(n, c))] for c in range(NL)]


def _thin(quarters, n):
    return [[q[(2 * i + 1) * len(q) // (2 * _per_quarter(n, c))] for i in range(_per_quarter(n, c))]
            for c, q in enumerate(quarters)]


class _Plan:
    def __init__(self, quarters, tiles, base):
        self.per = tiles // NL
        picked = [s for q in quarters for s in q]
        self.vpu = [tuple(hs for hs in range(HS) if (j, hs) in picked) for j in range(tiles)]
        self.stream = [[(j, hs) for j in range(c * self.per, (c + 1) * self.per) for hs in range(HS)
                        if (j, hs) not in picked] for c in range(NL)]
        self.groups = [len(s) // 2 for s in self.stream]
        self.first = [base + 8 * sum(self.groups[:c]) for c in range(NL)]


def _mxu_program(plans, n_dense, first):
    heads, per = len(plans), plans[0].per
    todo = [[(u, g) for u in range(heads) for g in range(plans[u].groups[(t + u) % NL])] for t in range(NL)]
    span = len(todo[0]) + heads * per + n_dense * W_SLOTS / NL
    start = sum(u < first for u, _ in todo[0]) + first * per
    due = [start + k * (span - start) / max(n_dense, 1) for k in range(n_dense + 1)]
    seqs = [[] for _ in range(NL)]
    issued = [[] for _ in range(NL)]
    time, done, taken, steps = [0] * NL, [0] * NL, [0] * NL, [0] * NL
    started, last_start = 0, -span

    def scores(t):
        u, g = todo[t][len(issued[t])]
        if seqs[t] and seqs[t][-1][0] == 'scores' and seqs[t][-1][2] == u:
            seqs[t][-1] = ('scores', seqs[t][-1][1] + 1, u, seqs[t][-1][3])
        else:
            seqs[t].append(('scores', 1, u, g))
        issued[t].append(time[t])
        time[t] += 1

    def covered(t, slots):
        return len(issued[t]) == len(todo[t]) or (seqs[t] and seqs[t][-1][1] >= slots)

    while min(steps) < heads * per:
        t = min((t for t in range(NL) if steps[t] < heads * per), key=lambda t: time[t])
        u, step = divmod(steps[t], per)
        done[t] += HS - len(plans[u].vpu[(t + u) % NL * per + step])
        last = (done[t] + 1) // 2 - 1
        closing = steps[t] == heads * per - 2
        while closing and len(issued[t]) < len(todo[t]):
            scores(t)
        while taken[t] < n_dense // NL:
            now = (taken[t] <= min(taken) + 1 and due[started] <= time[t] + MIN_RUN
                   and time[t] + MIN_RUN >= last_start + DENSE_GAP * (due[started + 1] - due[started]))
            if not (closing or (now and taken[t] < n_dense // NL - 1 and steps[t] > 0)):
                break
            while not covered(t, MIN_RUN):
                scores(t)
            seqs[t].append(('dense', W_SLOTS))
            last_start = time[t]
            time[t] += W_SLOTS
            taken[t] += 1
            started += 1
            if not closing:
                break
        wait = VALUE_DELAY + (STAGGER * t if steps[t] == 0 else 0)
        while len(issued[t]) < len(todo[t]) and (len(issued[t]) <= last or time[t] < issued[t][last] + wait
                                                 or not covered(t, 2)):
            scores(t)
        seqs[t].append(('values', 1, u, step))
        time[t] += 1
        steps[t] += 1
    assert started == n_dense
    free, merged = [0] * NL, []
    while any(seqs):
        t = min((t for t in range(NL) if seqs[t]), key=lambda t: free[t])
        op = seqs[t].pop(0)
        free[t] += op[1]
        merged.append((t,) + op)
    return merged


def _kernel(x_hbm, wq_hbm, wkt_hbm, wvt_hbm, wo_hbm, win_hbm, wsp_hbm, bsp_hbm, wout_hbm, c_hbm, wmod_hbm,
            out_hbm,
            x_v, wq_v, wkv_v, wo_v, win_v, wsp_v, bsp_v, wout_v, wmod_v,
            wq_s, wo_s, win_s, wout_s, wt_s, mod_s, row_s, h_s, kv_s, k_s, kn_s, kb_s, vt_s, qt_s, qf_s,
            o_s, h2_s, z2_s, bad_s, x1c_s, z2f_s, x1_s, z_s, g_s, out_v, c_v, zero_s, sems, wsems, osems):
    S, D = x_hbm.shape
    FH = wout_hbm.shape[0]
    H = HEADS
    DH = D // H
    NQ = S // T
    ND, NF = D // T, FH // T
    XT = NQ // NX

    def tile(i, n=T):
        return pl.ds(i * n if isinstance(i, int) else pl.multiple_of(i * n, n), n)

    def half(i):
        return tile(i, T // 2)

    def cp(src, dst, i):
        return pltpu.make_async_copy(src, dst, sems.at[i])

    c_cp = cp(c_hbm, c_v, 0)
    wmod_a = cp(wmod_hbm.at[:, pl.ds(0, 2 * D)], wmod_v.at[:, pl.ds(0, 2 * D)], 1)
    wq_cp = cp(wq_hbm, wq_v, 2)
    wk_cp = cp(wkt_hbm, wkv_v.at[pl.ds(0, DH), :], 3)
    wv_cp = cp(wvt_hbm, wkv_v.at[pl.ds(DH, DH), :], 4)
    wmod_b = cp(wmod_hbm.at[:, pl.ds(2 * D, 4 * D)], wmod_v.at[:, pl.ds(2 * D, 4 * D)], 5)
    wo_cp = cp(wo_hbm, wo_v.at[pl.ds(0, D), :], 6)
    win_cp = cp(win_hbm, win_v.at[pl.ds(0, D), :], 7)
    bsp_cp = cp(bsp_hbm, bsp_v, 8)
    wout_cp = cp(wout_hbm, wout_v, 9)

    def x_cp(b):
        return cp(x_hbm.at[tile(b, XT * T), :], x_v.at[tile(b, XT * T), pl.ds(0, D)], 10 + b)

    def wsp_cp(b):
        return pltpu.make_async_copy(wsp_hbm.at[:, tile(b, XT * T)], wsp_v.at[:, tile(b, XT * T)], wsems.at[b])

    def out_cp(m):
        return pltpu.make_async_copy(out_v.at[tile(m), :], out_hbm.at[tile(m), :], osems.at[m])

    for d in (c_cp, x_cp(0), wmod_a, wk_cp, wv_cp, *[x_cp(b) for b in range(1, NX)], wq_cp):
        d.start()

    def key0(j, hs):
        return j * T + (HS - 1 - hs) * 8

    quarters = _vpu_slots(VPU_SLOTS_MIXED, NQ)
    vidx = {s: i for i, s in enumerate(s for q in quarters for s in q)}
    mixed = _Plan(quarters, NQ, 0)
    plain = _Plan(_thin(quarters, VPU_SLOTS_PLAIN), NQ, S // 2)

    zero_s[0] = 0

    def fence(ref, value):
        ref[pl.ds(pl.multiple_of(ref.shape[0] - 8 + zero_s[0] * 8, 8), 8), 0:T] = value

    def stage(ref, k, value):
        ref[half(k), :] = value
        fence(ref, jnp.zeros((8, T), ref.dtype))

    def clear_gate():
        def clear(m, carry):
            g_s[m] = jnp.zeros((FH, T), f32)
            return carry
        lax.fori_loop(0, NQ, clear, 0)

    def normalise_x(b):
        x = x_v[tile(b, XT * T), 0:D].astype(f32)
        d = x - jnp.mean(x, axis=1, keepdims=True)
        return d * lax.rsqrt(jnp.mean(d * d, axis=1, keepdims=True) + EPS)

    def project_kv(b):
        kv_s[:, tile(b, XT * T)] = _dot_nt(wkv_v[...], _unpack(h_s[tile(b, XT * T // 2), :]))

    def arrange_keys():
        r = kv_s[...]
        vt_s[...] = _pack(r[DH:2 * DH])
        kn = jnp.concatenate([r[0:DH], jnp.zeros((T - DH, S), f32)], axis=0).astype(bf16).T
        kn_s[...] = pltpu.bitcast(kn, u32)
        kn = kn.astype(f32)

        def keys(slots):
            return jnp.concatenate([kn[key0(*slot):key0(*slot) + 8] for slot in slots], axis=0)

        for p in (mixed, plain):
            k_s[p.first[0]:p.first[0] + 8 * sum(p.groups), :] = pltpu.bitcast(
                keys([s for c in p.stream for s in c]).astype(bf16), u32)
        picked = keys(vidx)
        nm = DH // 2
        pick = (lax.broadcasted_iota(jnp.int32, (DH, nm * T), 0)
                == lax.broadcasted_iota(jnp.int32, (DH, nm * T), 1) // T).astype(f32)
        pick = jnp.concatenate([pick, jnp.zeros((T - DH, nm * T), f32)], axis=0).astype(bf16)
        wide = _dot(picked.astype(bf16), pick)
        for d in range(DH):
            for i in range(len(vidx)):
                rows = slice(8 * i, 8 * i + 8)
                kb_s[i, d] = (wide[rows, d * T:(d + 1) * T] if d < nm
                              else jnp.broadcast_to(picked[rows, d:d + 1], (8, T)))

    clear_gate()
    c_cp.wait()
    cf = c_v[...].astype(f32)
    sc = jnp.broadcast_to(cf * jax.nn.sigmoid(cf), (16, D)).astype(bf16)
    x_cp(0).wait()
    xn = normalise_x(0)
    wmod_a.wait()
    mod_a = _dot(sc, wmod_v[:, 0:2 * D])[0:1]
    shift, scale = mod_a[:, 0:D], 1.0 + mod_a[:, D:2 * D]
    h_s[tile(0, XT * T // 2), :] = _pack(xn * scale + shift)

    held, staging = [], []

    def accumulate(k, value):
        if k:
            value = value + held.pop()
        if k < ND - 1:
            held.append(value)
            return None
        if staging:
            staging.pop(0)(value)
        return value

    def query_products(i):
        def product(r, k):
            q = accumulate(k, _dot_nt(_unpack(wq_s[half(r), tile(k)]), _unpack(h_s[half(i), tile(k)])))
            if q is not None:
                q = q * ((DH ** -0.5) * math.log2(math.e))
                qt_s[half(r), :] = _pack(q)
                qf_s[tile(r), :] = q
        return [functools.partial(product, r, k) for r in range(ND) for k in range(ND)]

    def mixer_products(i, late=0):
        x1m, z2m, x1_stats, z2_stats = _Moments(), _Moments(), [], []

        def out_proj(n, k):
            a = accumulate(k, _dot(_unpack(wo_s[half(n), tile(k)]), _unpack(o_s[half(k), :])))
            if a is not None:
                x1 = x_v[tile(i), tile(n)].T.astype(f32) + mod_s[0, tile(n), :] * a
                x1c_s[tile(n), :] = x1
                x1_s[i, tile(n), :] = x1
                x1m.add(x1)
                if n == ND - 1:
                    x1_stats.extend(x1m.mean_rstd())
                    for a in range(ND - late):
                        modulate(a)
                    staging[:0] = [functools.partial(modulate, a) for a in range(ND - late, ND)]

        def modulate(k, token=None):
            if token is not None:
                fence(x1c_s, token[0:8])
            mean, rstd = x1_stats
            stage(h2_s, k, _pack((x1c_s[tile(k), :] - mean) * rstd * mod_s[2, tile(k), :] + mod_s[1, tile(k), :]))

        def normalise_z2(n):
            stage(z2_s, n, _pack((z2f_s[tile(n), :] - z2_stats[0]) * z2_stats[1]))

        def in_proj(n, k):
            z = accumulate(k, _dot(_unpack(win_s[half(n), tile(k)]), _unpack(h2_s[half(k), :])))
            if z is None:
                return
            z = _gelu_of_half(z)
            if n < NF:
                z_s[i, tile(n), :] = z
                if n < NF - 1:
                    fence(z2f_s, z[0:8])
                    normalise_z2(n + 1)
            else:
                z2f_s[tile(n - NF), :] = z
                z2m.add(z)
                if n == 2 * NF - 1:
                    z2_stats.extend(z2m.mean_rstd())
                    normalise_z2(0)
        return ([functools.partial(out_proj, n, k) for n in range(ND) for k in range(ND)],
                [functools.partial(in_proj, n, k) for n in (*range(NF, 2 * NF), *range(NF)) for k in range(ND)])

    def stage_wsp(i, m, token):
        wsp_v[0:16, pl.ds(pl.multiple_of(S + zero_s[0] * T, T), T)] = token[0:16].astype(bf16)
        wt_s[half(m), :] = pltpu.bitcast(wsp_v[tile(m), tile(i)].T, u32)
        if m == NQ - 1:
            fence(wt_s, jnp.zeros((8, T), u32))

    def spatial_products():
        def product(m, n):
            g_s[m, tile(n), :] += _dot(_unpack(z2_s[half(n), :]), _unpack(wt_s[half(m), :]))
        return [functools.partial(product, m, n) for m in range(NQ) for n in range(NF)]

    def run(products):
        for p in products:
            p()

    def padded_query(hd):
        return _unpack(jnp.concatenate([qt_s[tile(hd, DH // 2), :], jnp.zeros(((T - DH) // 2, T), u32)], axis=0))

    def attention(plans, dense=(), first=0, head0=0, side=()):
        dense, side = list(dense), list(side)
        n_side = 1.3 * len(side)
        q, rows, sums, accs, probs, closed = {}, {}, {}, {}, {}, {}

        def keep(u, t, slot, e):
            sums[u, t] = e if (u, t) not in sums else sums[u, t] + e
            probs[u, slot] = e

        def vpu_scores(u, t, slot):
            if u not in rows:
                qf = qf_s[tile(head0 + u + zero_s[0], DH), :]
                rows[u] = [jnp.broadcast_to(qf[d:d + 1], (8, T)) for d in range(DH)]
            part = [None, None]
            for d in range(DH):
                term = kb_s[vidx[slot], d] * rows[u][d]
                part[d % 2] = term if d < 2 else part[d % 2] + term
            keep(u, t, slot, jnp.exp2(part[0] + part[1]))

        def mxu_scores(t, n, u, g0):
            if u not in q:
                q[u] = padded_query(head0 + u)
            plan, c = plans[u], (t + u) % NL
            e = jnp.exp2(_dot(_unpack(k_s[plan.first[c] + 8 * g0:plan.first[c] + 8 * (g0 + n), :]), q[u]))
            for a in range(2 * n):
                keep(u, t, plan.stream[c][2 * g0 + a], e[a * 8:(a + 1) * 8])

        def values(t, u, step):
            plan = plans[u]
            j = (t + u) % NL * plan.per + step
            for hs in plan.vpu[j]:
                vpu_scores(u, t, (j, hs))
            p = jnp.concatenate([probs.pop((u, (j, hs))) for hs in reversed(range(HS))], axis=0)
            pv = _dot(_unpack(vt_s[:, tile(j)]), p.astype(bf16))
            accs[u] = pv if u not in accs else pv + accs[u]
            if side and t == 0 and (len(side) + 1) * len(plans) * plan.per > n_side * (
                    (len(plans) - u) * plan.per - step):
                side.pop(0)(pv)
            closed[u] = closed.get(u, 0) + 1
            if closed[u] == NQ:
                l = functools.reduce(lambda a, b: a + b, [sums.pop((u, c)) for c in range(NL)])
                l = jnp.sum(l, axis=0, keepdims=True)
                o = accs.pop(u) * (1.0 / l)
                size = jnp.abs(o)
                ok = (l >= L_MIN) & (l <= L_MAX) & (size[0:8] < jnp.inf) & (size[8:16] < jnp.inf)
                bad_s[...] = jnp.where(ok, bad_s[...], 1.0)
                o_s[tile(head0 + u, DH // 2), :] = _pack(o)

        for t, kind, n, *args in _mxu_program(plans, len(dense), first):
            if kind == 'dense':
                dense.pop(0)()
            elif kind == 'scores':
                mxu_scores(t, n, *args)
            else:
                values(t, *args)
        assert not side and not probs

    def normalise_block(b, carry):
        x_cp(b).wait()
        project_kv(b - 1)
        h_s[tile(b, XT * T // 2), :] = _pack(normalise_x(b) * scale + shift)
        return carry

    wk_cp.wait()
    wv_cp.wait()
    lax.fori_loop(1, NX, normalise_block, 0)
    for d in (wmod_b, wo_cp, win_cp):
        d.start()
    wq_cp.wait()
    wq_s[...] = pltpu.bitcast(wq_v[...].T, u32)
    project_kv(NX - 1)
    arrange_keys()
    run(query_products(0))
    bad_s[...] = jnp.zeros((8, T), f32)
    attention([plain] * FIRST_SPLIT)

    for d in (*[wsp_cp(b) for b in range(NX)], bsp_cp, wout_cp):
        d.start()
    for d in (wmod_b, wo_cp, win_cp):
        d.wait()
    mod_b = _dot(sc, wmod_v[:, 2 * D:5 * D])[0:1]
    row_s[0:1, :] = mod_b[:, 0:D]
    row_s[1:2, :] = 0.5 * mod_b[:, D:2 * D]
    row_s[2:3, :] = 0.5 * (1.0 + mod_b[:, 2 * D:3 * D])

    def spread(v, row):
        for n in range(ND):
            mod_s[v, tile(n), :] = jnp.broadcast_to(row[:, n * T:(n + 1) * T], (T, T)).T

    def spread_row(v, token):
        fence(row_s, token[0:8])
        spread(v, row_s[v:v + 1, :])

    def transpose(src, dst, n, token):
        src[pl.ds(pl.multiple_of(D + zero_s[0] * 16, 16), 16), 0:T] = token.astype(bf16)
        dst[half(n), :] = pltpu.bitcast(src[0:D, tile(n)].T, u32)

    attention([plain] * (H - FIRST_SPLIT), head0=FIRST_SPLIT,
              side=[functools.partial(spread_row, v) for v in range(3)]
              + [functools.partial(transpose, wo_v, wo_s, n) for n in range(ND)]
              + [functools.partial(transpose, win_v, win_s, n) for n in range(2 * NF)])

    def body(i, carry):
        @pl.when((i - 1) % XT == 0)
        def _():
            wsp_cp((i - 1) // XT).wait()

        out_proj, in_proj = mixer_products(i - 1, LATE_TILES)
        staging.extend(functools.partial(stage_wsp, i - 1, m) for m in range(NQ))
        run(out_proj + query_products(i) + in_proj)
        spatial = spatial_products()
        run(spatial[:EARLY_SPATIAL])
        attention([plain] * PLAIN_HEADS + [mixed] * (H - PLAIN_HEADS), spatial[EARLY_SPATIAL:], first=PLAIN_HEADS)
        return carry

    lax.fori_loop(1, NQ, body, 0)
    for b in range((NQ - 2) // XT + 1, NX):
        wsp_cp(b).wait()

    @pl.when(jnp.max(bad_s[...]) > 0.0)
    def _():
        clear_gate()

        def redo(i, carry):
            run(query_products(i))

            def head(hd, carry):
                s = _dot(_unpack(kn_s[...]), padded_query(hd))
                e = jnp.exp2(s - jnp.max(s, axis=0, keepdims=True))
                pv = _dot(_unpack(vt_s[...]), e.astype(bf16))
                o_s[tile(hd, DH // 2), :] = _pack(pv * (1.0 / jnp.sum(e, axis=0, keepdims=True)))
                return carry
            lax.fori_loop(0, H, head, 0)

            @pl.when(i < NQ - 1)
            def _():
                out_proj, in_proj = mixer_products(i)
                run(out_proj + in_proj)

                def spatial(m, carry):
                    g_s[m] += _dot_nt(_unpack(z2_s[0:FH // 2, :]), wsp_v[tile(m), tile(i)])
                    return carry
                lax.fori_loop(0, NQ, spatial, 0)
            return carry
        lax.fori_loop(0, NQ, redo, 0)

    bsp_cp.wait()
    wout_cp.wait()
    wout_s[...] = pltpu.bitcast(wout_v[...].T, u32)
    out_proj, in_proj = mixer_products(NQ - 1)
    staging.extend(functools.partial(stage_wsp, NQ - 1, m) for m in range(NQ))
    run(out_proj)
    spread(3, _dot(sc, wmod_v[:, 5 * D:6 * D])[0:1])
    run(in_proj)
    bias = bsp_v[...].astype(f32)
    for m in range(NQ):
        qf_s[tile(m, 8), :] = jnp.broadcast_to(bias[m:m + 1], (8, T))

    def gate(part, carry):
        for a in range(2):
            ms = [(part * 2 + a) * XT + j for j in range(XT)]
            g = _dot(_unpack(z2_s[0:FH // 2, :]), jnp.concatenate([_unpack(wt_s[half(m), :]) for m in ms], axis=1))
            u = []
            for j, m in enumerate(ms):
                prior = g_s[m].reshape(FH // 8, 8, T) + qf_s[tile(m, 8), :][None]
                u.append((z_s[m] * (g[:, j * T:(j + 1) * T] + prior.reshape(FH, T))).astype(bf16))
            y = _dot(_unpack(wout_s[...]), jnp.concatenate(u, axis=1))
            for j, m in enumerate(ms):
                out_v[tile(m), :] = (x1_s[m] + mod_s[3] * y[:, j * T:(j + 1) * T]).astype(bf16).T
                out_cp(m).start()
        return carry

    lax.fori_loop(0, NX // 2, gate, 0)
    for m in range(NQ):
        out_cp(m).wait()


@jax.jit
def pallas_adaLN_cond__grouped_kv_mqa__mixer_gmlp__prompt_kernel(
    A_x: jax.Array,
    A_wq: jax.Array,
    A_wk: jax.Array,
    A_wv: jax.Array,
    A_wo: jax.Array,
    B_x: jax.Array,
    B_w_in: jax.Array,
    B_w_sp: jax.Array,
    B_b_sp: jax.Array,
    B_w_out: jax.Array,
    c: jax.Array,
    w_mod: jax.Array,
):
    del B_x
    B, S, D = A_x.shape
    DH = D // HEADS
    FH = B_w_out.shape[0]
    NQ = S // T
    V = pltpu.VMEM
    dma = pltpu.SemaphoreType.DMA
    scratch = [
        V((S, D + T), bf16), V((D, D), bf16), V((2 * DH, D), bf16), V((D + 16, D), bf16),
        V((D + 16, 2 * FH), bf16), V((S, S + T), bf16), V((NQ, T), bf16), V((FH, D), bf16), V((D, 6 * D), bf16),
        V((D // 2, D), u32), V((D // 2, D), u32), V((FH, D), u32), V((D // 2, FH), u32), V((S // 2 + 8, T), u32),
        V((4, D, T), f32), V((16, D), f32), V((S // 2, D), u32), V((2 * DH, S), f32),
        V((S, T), u32), V((S // 2, T), u32), V((VPU_SLOTS_MIXED, DH, 8, T), f32), V((DH // 2, S), u32),
        V((D // 2, T), u32), V((D, T), f32),
        V((D // 2, T), u32), V((D // 2 + 8, T), u32), V((FH // 2 + 8, T), u32),
        V((8, T), f32), V((D + 8, T), f32), V((FH + 8, T), f32),
        V((NQ, D, T), f32), V((NQ, FH, T), f32), V((NQ, FH, T), f32), V((S, D), bf16),
        V((1, D), bf16), pltpu.SMEM((1,), jnp.int32),
        dma((10 + NX,)), dma((NX,)), dma((NQ,)),
    ]
    out = pl.pallas_call(
        _kernel,
        out_shape=jax.ShapeDtypeStruct((S, D), A_x.dtype),
        in_specs=[pl.BlockSpec(memory_space=pl.ANY)] * 11,
        out_specs=pl.BlockSpec(memory_space=pl.ANY),
        scratch_shapes=scratch,
        compiler_params=pltpu.CompilerParams(
            vmem_limit_bytes=100 * 2**20, flags={'XLA_TPU_EVENLY_DISTRIBUTE_CRITICAL_NODES': True}),
        name='fused',
    )(A_x.reshape(S, D), A_wq, A_wk.T, A_wv.T, A_wo, B_w_in, B_w_sp, B_b_sp.reshape(NQ, T), B_w_out, c, w_mod)
    return out.reshape(B, S, D)
```

```python
import functools
import math

import jax
import jax.numpy as jnp
from jax import lax
import jax.experimental.pallas as pl
import jax.experimental.pallas.tpu as pltpu

f32, bf16, u32 = jnp.float32, jnp.bfloat16, jnp.uint32

HEADS = 32
EPS = 1e-5
T = 128
NL = 4
HS = T // 8
W_SLOTS = T // 16
NX = 4
L_MIN, L_MAX = 2.0 ** -40, 2.0 ** 80

VPU_SLOTS_MIXED = 52
VPU_SLOTS_PLAIN = 42
PLAIN_HEADS = 11
EARLY_SPATIAL = 8
VALUE_DELAY = 10
MIN_RUN = 4
STAGGER = 2
DENSE_GAP = 0.7
LATE_TILES = 3
FIRST_SPLIT = 24


def _pack(x):
    if x.shape[1] != T:
        return pltpu.bitcast(x.astype(bf16), u32)
    h = x.shape[0] // 2
    if h % 16:
        return _pack(jnp.concatenate([x, x], axis=1))[:, :T]
    y = _pack(jnp.concatenate([x[:h], x[h:]], axis=1))
    return jnp.concatenate([y[:, :T], y[:, T:]], axis=0)


def _unpack(x):
    return pltpu.bitcast(x, bf16)


def _dot(a, b):
    return jnp.dot(a, b, preferred_element_type=f32)


def _dot_nt(a, b):
    return lax.dot_general(a, b, (((1,), (1,)), ((), ())), preferred_element_type=f32)


def _gelu_of_half(hx):
    c0 = 2.0 * math.sqrt(2.0 / math.pi)
    return hx + hx * jnp.tanh(hx * (c0 + (4.0 * 0.044715 * c0) * (hx * hx)))


class _Moments:
    def __init__(self):
        self.n = 0

    def add(self, x):
        for r in range(0, x.shape[0], 8):
            v = x[r:r + 8]
            if self.n == 0:
                self.pivot = v
            else:
                d = v - self.pivot
                self.s1 = d if self.n == 1 else self.s1 + d
                self.s2 = d * d if self.n == 1 else self.s2 + d * d
            self.n += 1

    def mean_rstd(self):
        off = self.s1 * (1.0 / self.n)
        part = self.pivot + off
        mean = jnp.sum(part, axis=0, keepdims=True) * 0.125
        d = part - mean
        m2 = (self.s2 * (1.0 / self.n) - off * off) + d * d
        var = jnp.maximum(jnp.sum(m2, axis=0, keepdims=True) * 0.125, 0.0)
        return mean, lax.rsqrt(var + EPS)


def _per_quarter(n, c):
    return (n // 2 * (c + 1)) // NL * 2 - (n // 2 * c) // NL * 2


def _vpu_slots(n, tiles):
    per = tiles // NL * HS
    return [[divmod(c * per + int((i + c / NL) * per / _per_quarter(n, c)), HS)
             for i in range(_per_quarter(n, c))] for c in range(NL)]


def _thin(quarters, n):
    return [[q[(2 * i + 1) * len(q) // (2 * _per_quarter(n, c))] for i in range(_per_quarter(n, c))]
            for c, q in enumerate(quarters)]


class _Plan:
    def __init__(self, quarters, tiles, base):
        self.per = tiles // NL
        picked = [s for q in quarters for s in q]
        self.vpu = [tuple(hs for hs in range(HS) if (j, hs) in picked) for j in range(tiles)]
        self.stream = [[(j, hs) for j in range(c * self.per, (c + 1) * self.per) for hs in range(HS)
                        if (j, hs) not in picked] for c in range(NL)]
        self.groups = [len(s) // 2 for s in self.stream]
        self.first = [base + 8 * sum(self.groups[:c]) for c in range(NL)]


def _mxu_program(plans, n_dense, first):
    heads, per = len(plans), plans[0].per
    todo = [[(u, g) for u in range(heads) for g in range(plans[u].groups[(t + u) % NL])] for t in range(NL)]
    span = len(todo[0]) + heads * per + n_dense * W_SLOTS / NL
    start = sum(u < first for u, _ in todo[0]) + first * per
    due = [start + k * (span - start) / max(n_dense, 1) for k in range(n_dense + 1)]
    seqs = [[] for _ in range(NL)]
    issued = [[] for _ in range(NL)]
    time, done, taken, steps = [0] * NL, [0] * NL, [0] * NL, [0] * NL
    started, last_start = 0, -span

    def scores(t):
        u, g = todo[t][len(issued[t])]
        if seqs[t] and seqs[t][-1][0] == 'scores' and seqs[t][-1][2] == u:
            seqs[t][-1] = ('scores', seqs[t][-1][1] + 1, u, seqs[t][-1][3])
        else:
            seqs[t].append(('scores', 1, u, g))
        issued[t].append(time[t])
        time[t] += 1

    def covered(t, slots):
        return len(issued[t]) == len(todo[t]) or (seqs[t] and seqs[t][-1][1] >= slots)

    while min(steps) < heads * per:
        t = min((t for t in range(NL) if steps[t] < heads * per), key=lambda t: time[t])
        u, step = divmod(steps[t], per)
        done[t] += HS - len(plans[u].vpu[(t + u) % NL * per + step])
        last = (done[t] + 1) // 2 - 1
        closing = steps[t] == heads * per - 2
        while closing and len(issued[t]) < len(todo[t]):
            scores(t)
        while taken[t] < n_dense // NL:
            now = (taken[t] <= min(taken) + 1 and due[started] <= time[t] + MIN_RUN
                   and time[t] + MIN_RUN >= last_start + DENSE_GAP * (due[started + 1] - due[started]))
            if not (closing or (now and taken[t] < n_dense // NL - 1 and steps[t] > 0)):
                break
            while not covered(t, MIN_RUN):
                scores(t)
            seqs[t].append(('dense', W_SLOTS))
            last_start = time[t]
            time[t] += W_SLOTS
            taken[t] += 1
            started += 1
            if not closing:
                break
        wait = VALUE_DELAY + (STAGGER * t if steps[t] == 0 else 0)
        while len(issued[t]) < len(todo[t]) and (len(issued[t]) <= last or time[t] < issued[t][last] + wait
                                                 or not covered(t, 2)):
            scores(t)
        seqs[t].append(('values', 1, u, step))
        time[t] += 1
        steps[t] += 1
    assert started == n_dense
    free, merged = [0] * NL, []
    while any(seqs):
        t = min((t for t in range(NL) if seqs[t]), key=lambda t: free[t])
        op = seqs[t].pop(0)
        free[t] += op[1]
        merged.append((t,) + op)
    return merged


def _kernel(x_hbm, wq_hbm, wkt_hbm, wvt_hbm, wo_hbm, win_hbm, wsp_hbm, bsp_hbm, wout_hbm, c_hbm, wmod_hbm,
            out_hbm,
            x_v, wq_v, wkv_v, wo_v, win_v, wsp_v, bsp_v, wout_v, wmod_v,
            wq_s, wo_s, win_s, wout_s, wt_s, mod_s, row_s, h_s, kv_s, k_s, kn_s, kb_s, vt_s, qt_s, qf_s,
            o_s, h2_s, z2_s, bad_s, x1c_s, z2f_s, x1_s, z_s, g_s, out_v, c_v, zero_s, sems, wsems, osems):
    S, D = x_hbm.shape
    FH = wout_hbm.shape[0]
    H = HEADS
    DH = D // H
    NQ = S // T
    ND, NF = D // T, FH // T
    XT = NQ // NX

    def tile(i, n=T):
        return pl.ds(i * n if isinstance(i, int) else pl.multiple_of(i * n, n), n)

    def half(i):
        return tile(i, T // 2)

    def cp(src, dst, i):
        return pltpu.make_async_copy(src, dst, sems.at[i])

    c_cp = cp(c_hbm, c_v, 0)
    wmod_a = cp(wmod_hbm.at[:, pl.ds(0, 2 * D)], wmod_v.at[:, pl.ds(0, 2 * D)], 1)
    wq_cp = cp(wq_hbm, wq_v, 2)
    wk_cp = cp(wkt_hbm, wkv_v.at[pl.ds(0, DH), :], 3)
    wv_cp = cp(wvt_hbm, wkv_v.at[pl.ds(DH, DH), :], 4)
    wmod_b = cp(wmod_hbm.at[:, pl.ds(2 * D, 4 * D)], wmod_v.at[:, pl.ds(2 * D, 4 * D)], 5)
    wo_cp = cp(wo_hbm, wo_v.at[pl.ds(0, D), :], 6)
    win_cp = cp(win_hbm, win_v.at[pl.ds(0, D), :], 7)
    bsp_cp = cp(bsp_hbm, bsp_v, 8)
    wout_cp = cp(wout_hbm, wout_v, 9)

    def x_cp(b):
        return cp(x_hbm.at[tile(b, XT * T), :], x_v.at[tile(b, XT * T), pl.ds(0, D)], 10 + b)

    def wsp_cp(b):
        return pltpu.make_async_copy(wsp_hbm.at[:, tile(b, XT * T)], wsp_v.at[:, tile(b, XT * T)], wsems.at[b])

    def out_cp(m):
        return pltpu.make_async_copy(out_v.at[tile(m), :], out_hbm.at[tile(m), :], osems.at[m])

    for d in (c_cp, x_cp(0), wmod_a, wk_cp, wv_cp, *[x_cp(b) for b in range(1, NX)], wq_cp):
        d.start()

    def key0(j, hs):
        return j * T + (HS - 1 - hs) * 8

    quarters = _vpu_slots(VPU_SLOTS_MIXED, NQ)
    vidx = {s: i for i, s in enumerate(s for q in quarters for s in q)}
    mixed = _Plan(quarters, NQ, 0)
    plain = _Plan(_thin(quarters, VPU_SLOTS_PLAIN), NQ, S // 2)

    zero_s[0] = 0

    def fence(ref, value):
        ref[pl.ds(pl.multiple_of(ref.shape[0] - 8 + zero_s[0] * 8, 8), 8), 0:T] = value

    def stage(ref, k, value):
        ref[half(k), :] = value
        fence(ref, jnp.zeros((8, T), ref.dtype))

    def clear_gate():
        def clear(m, carry):
            g_s[m] = jnp.zeros((FH, T), f32)
            return carry
        lax.fori_loop(0, NQ, clear, 0)

    def normalise_x(b):
        x = x_v[tile(b, XT * T), 0:D].astype(f32)
        d = x - jnp.mean(x, axis=1, keepdims=True)
        return d * lax.rsqrt(jnp.mean(d * d, axis=1, keepdims=True) + EPS)

    def project_kv(b):
        kv_s[:, tile(b, XT * T)] = _dot_nt(wkv_v[...], _unpack(h_s[tile(b, XT * T // 2), :]))

    def arrange_keys():
        r = kv_s[...]
        vt_s[...] = _pack(r[DH:2 * DH])
        kn = jnp.concatenate([r[0:DH], jnp.zeros((T - DH, S), f32)], axis=0).astype(bf16).T
        kn_s[...] = pltpu.bitcast(kn, u32)
        kn = kn.astype(f32)

        def keys(slots):
            return jnp.concatenate([kn[key0(*slot):key0(*slot) + 8] for slot in slots], axis=0)

        for p in (mixed, plain):
            k_s[p.first[0]:p.first[0] + 8 * sum(p.groups), :] = pltpu.bitcast(
                keys([s for c in p.stream for s in c]).astype(bf16), u32)
        picked = keys(vidx)
        nm = DH // 2
        pick = (lax.broadcasted_iota(jnp.int32, (DH, nm * T), 0)
                == lax.broadcasted_iota(jnp.int32, (DH, nm * T), 1) // T).astype(f32)
        pick = jnp.concatenate([pick, jnp.zeros((T - DH, nm * T), f32)], axis=0).astype(bf16)
        wide = _dot(picked.astype(bf16), pick)
        for d in range(DH):
            for i in range(len(vidx)):
                rows = slice(8 * i, 8 * i + 8)
                kb_s[i, d] = (wide[rows, d * T:(d + 1) * T] if d < nm
                              else jnp.broadcast_to(picked[rows, d:d + 1], (8, T)))

    clear_gate()
    c_cp.wait()
    cf = c_v[...].astype(f32)
    sc = jnp.broadcast_to(cf * jax.nn.sigmoid(cf), (16, D)).astype(bf16)
    x_cp(0).wait()
    xn = normalise_x(0)
    wmod_a.wait()
    mod_a = _dot(sc, wmod_v[:, 0:2 * D])[0:1]
    shift, scale = mod_a[:, 0:D], 1.0 + mod_a[:, D:2 * D]
    h_s[tile(0, XT * T // 2), :] = _pack(xn * scale + shift)

    held, staging = [], []

    def accumulate(k, value):
        if k:
            value = value + held.pop()
        if k < ND - 1:
            held.append(value)
            return None
        if staging:
            staging.pop(0)(value)
        return value

    def query_products(i):
        def product(r, k):
            q = accumulate(k, _dot_nt(_unpack(wq_s[half(r), tile(k)]), _unpack(h_s[half(i), tile(k)])))
            if q is not None:
                q = q * ((DH ** -0.5) * math.log2(math.e))
                qt_s[half(r), :] = _pack(q)
                qf_s[tile(r), :] = q
        return [functools.partial(product, r, k) for r in range(ND) for k in range(ND)]

    def mixer_products(i, late=0):
        x1m, z2m, x1_stats, z2_stats = _Moments(), _Moments(), [], []

        def out_proj(n, k):
            a = accumulate(k, _dot(_unpack(wo_s[half(n), tile(k)]), _unpack(o_s[half(k), :])))
            if a is not None:
                x1 = x_v[tile(i), tile(n)].T.astype(f32) + mod_s[0, tile(n), :] * a
                x1c_s[tile(n), :] = x1
                x1_s[i, tile(n), :] = x1
                x1m.add(x1)
                if n == ND - 1:
                    x1_stats.extend(x1m.mean_rstd())
                    for f in range(ND - late):
                        modulate(f)
                    staging[:0] = [functools.partial(modulate, f) for f in range(ND - late, ND)]

        def modulate(k, token=None):
            if token is not None:
                fence(x1c_s, token[0:8])
            mean, rstd = x1_stats
            stage(h2_s, k, _pack((x1c_s[tile(k), :] - mean) * rstd * mod_s[2, tile(k), :] + mod_s[1, tile(k), :]))

        def normalise_z2(n):
            stage(z2_s, n, _pack((z2f_s[tile(n), :] - z2_stats[0]) * z2_stats[1]))

        def in_proj(n, k):
            z = accumulate(k, _dot(_unpack(win_s[half(n), tile(k)]), _unpack(h2_s[half(k), :])))
            if z is None:
                return
            z = _gelu_of_half(z)
            if n < NF:
                z_s[i, tile(n), :] = z
                if n < NF - 1:
                    fence(z2f_s, z[0:8])
                    normalise_z2(n + 1)
            else:
                z2f_s[tile(n - NF), :] = z
                z2m.add(z)
                if n == 2 * NF - 1:
                    z2_stats.extend(z2m.mean_rstd())
                    normalise_z2(0)
        return ([functools.partial(out_proj, n, k) for n in range(ND) for k in range(ND)],
                [functools.partial(in_proj, n, k) for n in (*range(NF, 2 * NF), *range(NF)) for k in range(ND)])

    def stage_wsp(i, m, token):
        wsp_v[0:16, pl.ds(pl.multiple_of(S + zero_s[0] * T, T), T)] = token[0:16].astype(bf16)
        wt_s[half(m), :] = pltpu.bitcast(wsp_v[tile(m), tile(i)].T, u32)
        if m == NQ - 1:
            fence(wt_s, jnp.zeros((8, T), u32))

    def spatial_products():
        def product(m, n):
            g_s[m, tile(n), :] += _dot(_unpack(z2_s[half(n), :]), _unpack(wt_s[half(m), :]))
        return [functools.partial(product, m, n) for m in range(NQ) for n in range(NF)]

    def run(products):
        for p in products:
            p()

    def padded_query(hd):
        return _unpack(jnp.concatenate([qt_s[tile(hd, DH // 2), :], jnp.zeros(((T - DH) // 2, T), u32)], axis=0))

    def attention(plans, dense=(), first=0, head0=0, side=()):
        dense, side = list(dense), list(side)
        n_side = 1.3 * len(side)
        q, rows, sums, accs, probs, closed = {}, {}, {}, {}, {}, {}

        def keep(u, t, slot, e):
            sums[u, t] = e if (u, t) not in sums else sums[u, t] + e
            probs[u, slot] = e

        def vpu_scores(u, t, slot):
            if u not in rows:
                qf = qf_s[tile(head0 + u + zero_s[0], DH), :]
                rows[u] = [jnp.broadcast_to(qf[d:d + 1], (8, T)) for d in range(DH)]
            part = [None, None]
            for d in range(DH):
                term = kb_s[vidx[slot], d] * rows[u][d]
                part[d % 2] = term if d < 2 else part[d % 2] + term
            keep(u, t, slot, jnp.exp2(part[0] + part[1]))

        def mxu_scores(t, n, u, g0):
            if u not in q:
                q[u] = padded_query(head0 + u)
            plan, c = plans[u], (t + u) % NL
            e = jnp.exp2(_dot(_unpack(k_s[plan.first[c] + 8 * g0:plan.first[c] + 8 * (g0 + n), :]), q[u]))
            for a in range(2 * n):
                keep(u, t, plan.stream[c][2 * g0 + a], e[a * 8:(a + 1) * 8])

        def values(t, u, step):
            plan = plans[u]
            j = (t + u) % NL * plan.per + step
            for hs in plan.vpu[j]:
                vpu_scores(u, t, (j, hs))
            p = jnp.concatenate([probs.pop((u, (j, hs))) for hs in reversed(range(HS))], axis=0)
            pv = _dot(_unpack(vt_s[:, tile(j)]), p.astype(bf16))
            accs[u] = pv if u not in accs else pv + accs[u]
            if side and t == 0 and (len(side) + 1) * len(plans) * plan.per > n_side * (
                    (len(plans) - u) * plan.per - step):
                side.pop(0)(pv)
            closed[u] = closed.get(u, 0) + 1
            if closed[u] == NQ:
                l = functools.reduce(lambda a, b: a + b, [sums.pop((u, c)) for c in range(NL)])
                l = jnp.sum(l, axis=0, keepdims=True)
                o = accs.pop(u) * (1.0 / l)
                size = jnp.abs(o)
                ok = (l >= L_MIN) & (l <= L_MAX) & (size[0:8] < jnp.inf) & (size[8:16] < jnp.inf)
                bad_s[...] = jnp.where(ok, bad_s[...], 1.0)
                o_s[tile(head0 + u, DH // 2), :] = _pack(o)

        for t, kind, n, *args in _mxu_program(plans, len(dense), first):
            if kind == 'dense':
                dense.pop(0)()
            elif kind == 'scores':
                mxu_scores(t, n, *args)
            else:
                values(t, *args)
        assert not side and not probs

    def normalise_block(b, carry):
        x_cp(b).wait()
        project_kv(b - 1)
        h_s[tile(b, XT * T // 2), :] = _pack(normalise_x(b) * scale + shift)
        return carry

    wk_cp.wait()
    wv_cp.wait()
    lax.fori_loop(1, NX, normalise_block, 0)
    for d in (wmod_b, wo_cp, win_cp):
        d.start()
    wq_cp.wait()
    wq_s[...] = pltpu.bitcast(wq_v[...].T, u32)
    project_kv(NX - 1)
    arrange_keys()
    run(query_products(0))
    bad_s[...] = jnp.zeros((8, T), f32)
    attention([plain] * FIRST_SPLIT)

    for d in (*[wsp_cp(b) for b in range(NX)], bsp_cp, wout_cp):
        d.start()
    for d in (wmod_b, wo_cp, win_cp):
        d.wait()
    mod_b = _dot(sc, wmod_v[:, 2 * D:5 * D])[0:1]
    row_s[0:1, :] = mod_b[:, 0:D]
    row_s[1:2, :] = 0.5 * mod_b[:, D:2 * D]
    row_s[2:3, :] = 0.5 * (1.0 + mod_b[:, 2 * D:3 * D])

    def spread(v, row):
        for n in range(ND):
            mod_s[v, tile(n), :] = jnp.broadcast_to(row[:, n * T:(n + 1) * T], (T, T)).T

    def spread_row(v, token):
        fence(row_s, token[0:8])
        spread(v, row_s[v:v + 1, :])

    def transpose(src, dst, n, token):
        src[pl.ds(pl.multiple_of(D + zero_s[0] * 16, 16), 16), 0:T] = token.astype(bf16)
        dst[half(n), :] = pltpu.bitcast(src[0:D, tile(n)].T, u32)

    attention([plain] * (H - FIRST_SPLIT), head0=FIRST_SPLIT,
              side=[functools.partial(spread_row, v) for v in range(3)]
              + [functools.partial(transpose, wo_v, wo_s, n) for n in range(ND)]
              + [functools.partial(transpose, win_v, win_s, n) for n in range(2 * NF)])

    def body(i, carry):
        @pl.when((i - 1) % XT == 0)
        def _():
            wsp_cp((i - 1) // XT).wait()

        out_proj, in_proj = mixer_products(i - 1, LATE_TILES)
        staging.extend(functools.partial(stage_wsp, i - 1, m) for m in range(NQ))
        run(out_proj + query_products(i) + in_proj)
        assert not staging
        spatial = spatial_products()
        run(spatial[:EARLY_SPATIAL])
        attention([plain] * PLAIN_HEADS + [mixed] * (H - PLAIN_HEADS), spatial[EARLY_SPATIAL:], first=PLAIN_HEADS)
        return carry

    lax.fori_loop(1, NQ, body, 0)
    for b in range((NQ - 2) // XT + 1, NX):
        wsp_cp(b).wait()

    @pl.when(jnp.max(bad_s[...]) > 0.0)
    def _():
        clear_gate()

        def redo(i, carry):
            run(query_products(i))

            def head(hd, carry):
                s = _dot(_unpack(kn_s[...]), padded_query(hd))
                e = jnp.exp2(s - jnp.max(s, axis=0, keepdims=True))
                pv = _dot(_unpack(vt_s[...]), e.astype(bf16))
                o_s[tile(hd, DH // 2), :] = _pack(pv * (1.0 / jnp.sum(e, axis=0, keepdims=True)))
                return carry
            lax.fori_loop(0, H, head, 0)

            @pl.when(i < NQ - 1)
            def _():
                out_proj, in_proj = mixer_products(i)
                run(out_proj + in_proj)

                def spatial(m, carry):
                    g_s[m] += _dot_nt(_unpack(z2_s[0:FH // 2, :]), wsp_v[tile(m), tile(i)])
                    return carry
                lax.fori_loop(0, NQ, spatial, 0)
            return carry
        lax.fori_loop(0, NQ, redo, 0)

    bsp_cp.wait()
    wout_cp.wait()
    wout_s[...] = pltpu.bitcast(wout_v[...].T, u32)
    out_proj, in_proj = mixer_products(NQ - 1)
    staging.extend(functools.partial(stage_wsp, NQ - 1, m) for m in range(NQ))
    run(out_proj)
    spread(3, _dot(sc, wmod_v[:, 5 * D:6 * D])[0:1])
    run(in_proj)
    assert not staging
    bias = bsp_v[...].astype(f32)
    for m in range(NQ):
        qf_s[tile(m, 8), :] = jnp.broadcast_to(bias[m:m + 1], (8, T))

    def gate(part, carry):
        for a in range(2):
            ms = [(part * 2 + a) * XT + j for j in range(XT)]
            g = _dot(_unpack(z2_s[0:FH // 2, :]), jnp.concatenate([_unpack(wt_s[half(m), :]) for m in ms], axis=1))
            u = []
            for j, m in enumerate(ms):
                prior = g_s[m].reshape(FH // 8, 8, T) + qf_s[tile(m, 8), :][None]
                u.append((z_s[m] * (g[:, j * T:(j + 1) * T] + prior.reshape(FH, T))).astype(bf16))
            y = _dot(_unpack(wout_s[...]), jnp.concatenate(u, axis=1))
            for j, m in enumerate(ms):
                out_v[tile(m), :] = (x1_s[m] + mod_s[3] * y[:, j * T:(j + 1) * T]).astype(bf16).T
                out_cp(m).start()
        return carry

    lax.fori_loop(0, NX // 2, gate, 0)
    for m in range(NQ):
        out_cp(m).wait()


@jax.jit
def pallas_adaLN_cond__grouped_kv_mqa__mixer_gmlp__prompt_kernel(
    A_x: jax.Array,
    A_wq: jax.Array,
    A_wk: jax.Array,
    A_wv: jax.Array,
    A_wo: jax.Array,
    B_x: jax.Array,
    B_w_in: jax.Array,
    B_w_sp: jax.Array,
    B_b_sp: jax.Array,
    B_w_out: jax.Array,
    c: jax.Array,
    w_mod: jax.Array,
):
    del B_x
    B, S, D = A_x.shape
    DH = D // HEADS
    FH = B_w_out.shape[0]
    NQ = S // T
    V = pltpu.VMEM
    dma = pltpu.SemaphoreType.DMA
    scratch = [
        V((S, D + T), bf16), V((D, D), bf16), V((2 * DH, D), bf16), V((D + 16, D), bf16),
        V((D + 16, 2 * FH), bf16), V((S, S + T), bf16), V((NQ, T), bf16), V((FH, D), bf16), V((D, 6 * D), bf16),
        V((D // 2, D), u32), V((D // 2, D), u32), V((FH, D), u32), V((D // 2, FH), u32), V((S // 2 + 8, T), u32),
        V((4, D, T), f32), V((16, D), f32), V((S // 2, D), u32), V((2 * DH, S), f32),
        V((S, T), u32), V((S // 2, T), u32), V((VPU_SLOTS_MIXED, DH, 8, T), f32), V((DH // 2, S), u32),
        V((D // 2, T), u32), V((D, T), f32),
        V((D // 2, T), u32), V((D // 2 + 8, T), u32), V((FH // 2 + 8, T), u32),
        V((8, T), f32), V((D + 8, T), f32), V((FH + 8, T), f32),
        V((NQ, D, T), f32), V((NQ, FH, T), f32), V((NQ, FH, T), f32), V((S, D), bf16),
        V((1, D), bf16), pltpu.SMEM((1,), jnp.int32),
        dma((10 + NX,)), dma((NX,)), dma((NQ,)),
    ]
    out = pl.pallas_call(
        _kernel,
        out_shape=jax.ShapeDtypeStruct((S, D), A_x.dtype),
        in_specs=[pl.BlockSpec(memory_space=pl.ANY)] * 11,
        out_specs=pl.BlockSpec(memory_space=pl.ANY),
        scratch_shapes=scratch,
        compiler_params=pltpu.CompilerParams(
            vmem_limit_bytes=100 * 2**20, flags={'XLA_TPU_EVENLY_DISTRIBUTE_CRITICAL_NODES': True}),
        name='fused',
    )(A_x.reshape(S, D), A_wq, A_wk.T, A_wv.T, A_wo, B_w_in, B_w_sp, B_b_sp.reshape(NQ, T), B_w_out, c, w_mod)
    return out.reshape(B, S, D)
```
